```python
import jax
import jax.numpy as jnp

def _softmax(x, axis=-1):
    return jax.nn.softmax(x, axis=axis)
def _gelu(x):
    return jax.nn.gelu(x, approximate=True)
def _silu(x):
    return jax.nn.silu(x)
def _sigmoid(x):
    return jax.nn.sigmoid(x)
def _layernorm(x, axis=-1, eps=1e-5):
    m = jnp.mean(x, axis=axis, keepdims=True)
    v = jnp.var(x, axis=axis, keepdims=True)
    return (x - m) / jnp.sqrt(v + eps)
def _scatter_add(tgt, idx, src, axis=0):
    return tgt.at[idx].add(src)
def _segment_sum(src, seg, n):
    return jax.ops.segment_sum(src, seg, n)
class _Rng:
    def __init__(self, key):
        self._k = key
    def _next(self):
        self._k, sub = jax.random.split(self._k)
        return sub
    def normal(self, shape):
        return jax.random.normal(self._next(), shape, dtype=jnp.bfloat16)
    def randint(self, lo, hi, shape):
        return jax.random.randint(self._next(), shape, lo, hi, dtype=jnp.int32)
    def uniform(self, shape, lo=0.0, hi=1.0):
        return jax.random.uniform(self._next(), shape, jnp.bfloat16, lo, hi)
    def permutation(self, n):
        return jax.random.permutation(self._next(), n)


kernel_name = 'gated_mix__ssm_conv_h3__sliding_local_dilated__prompt'

def setup_inputs():
    _rng = _Rng(jax.random.key(int.from_bytes(__import__("os").urandom(4), "little")))
    _w = (lambda a: (lambda t: t.astype(jnp.bfloat16) if jnp.issubdtype(t.dtype, jnp.floating) else t)(jnp.asarray(a)))
    def _A_setup():
        B, S, D = 1, 2048, 640
        ks = 4
        return {
            "q": _w((lambda *s: _rng.normal(s) * 0.05)(B, S, D)),
            "k": _w((lambda *s: _rng.normal(s) * 0.05)(B, S, D)),
            "v": _w((lambda *s: _rng.normal(s) * 0.05)(B, S, D)),
            "shift_k": _w((lambda *s: _rng.normal(s) * 0.05)(D, ks) * 0.5),
            "ssm_k": _w((lambda *s: _rng.normal(s) * 0.05)(D, S) * (1.0 / S ** 0.5)),
            "ssm_D": _w((lambda *s: _rng.normal(s) * 0.05)(D)),
        }
    _A_in = _A_setup()

    def _B_setup():
        B, S, D = 1, 2048, 640
        return {
            "x": _w((lambda *s: _rng.normal(s) * 0.05)(B, S, D)),
            "wqkv": _w((lambda *s: _rng.normal(s) * 0.05)(D, 3 * D)),
            "wo": _w((lambda *s: _rng.normal(s) * 0.05)(D, D)),
        }
    _B_in = _B_setup()

    return {
        "A_q": _A_in["q"],
        "A_k": _A_in["k"],
        "A_v": _A_in["v"],
        "A_shift_k": _A_in["shift_k"],
        "A_ssm_k": _A_in["ssm_k"],
        "A_ssm_D": _A_in["ssm_D"],
        "B_x": _B_in["x"],
        "B_wqkv": _B_in["wqkv"],
        "B_wo": _B_in["wo"],
        "gate_w": _w((lambda *s: _rng.normal(s) * 0.05)(640)),
    }

def reference(A_q, A_k, A_v, A_shift_k, A_ssm_k, A_ssm_D, B_x, B_wqkv, B_wo, gate_w):
    def _A_ref(q, k, v, shift_k, ssm_k, ssm_D):
        B, S, D = q.shape
        ks = shift_k.shape[-1]
        k_pad = jnp.pad(k, ((0, 0), (ks - 1, 0), (0, 0)))
        k_shift = jnp.zeros_like(k)
        for t in range(ks):
            k_shift = k_shift + k_pad[:, t:t + S, :] * shift_k[:, ks - 1 - t][None, None, :]
        kv = k_shift * v
        L = 2 * S
        kv_pad = jnp.pad(kv, ((0, 0), (0, S), (0, 0)))
        kf_pad = jnp.pad(ssm_k, ((0, 0), (0, S)))
        kv_f = (lambda x, axes=(-2,-1): jnp.fft.rfft2(x.astype(jnp.float32), axes=axes))(kv_pad[:, None, :, :], axes=(1, 2))
        kf_f = (lambda x, axes=(-2,-1): jnp.fft.rfft2(x.astype(jnp.float32), axes=axes))(kf_pad[:, None, :], axes=(1, 2))
        kf_f = (lambda x, *d: x.transpose(*d))(kf_f, 1, 2, 0)
        y_f = kv_f * kf_f[None, :, :, :]
        y = (lambda x, s, axes=(-2,-1): jnp.fft.irfft2(x, s=s, axes=axes).astype(jnp.bfloat16))(y_f, (1, L), axes=(1, 2))[:, 0, :S, :]
        y = y + kv * ssm_D[None, None, :]
        return q * y

    def _B_ref(x, wqkv, wo):
        B, S, D = x.shape
        H = 32; Dh = D // H
        W, dil = 8, 2
        qkv = (lambda x, *d: x.transpose(*d))((x @ wqkv).reshape(B, S, 3, H, Dh), 2, 0, 3, 1, 4)
        q, k, v = qkv[0], qkv[1], qkv[2]
        scale = Dh ** -0.5
        pos = jnp.arange(S)
        off = jnp.arange(W) * dil
        idx = pos[:, None] - off[None, :]
        mask = idx >= 0
        idx_c = jnp.where(mask, idx, 0).reshape(-1)
        kg = k[:, :, idx_c, :].reshape(B, H, S, W, Dh)
        vg = v[:, :, idx_c, :].reshape(B, H, S, W, Dh)
        logits = jnp.einsum("bhsd,bhswd->bhsw", q, kg) * scale
        logits = jnp.where(mask[None, None, :, :], logits, -1e9)
        attn = _softmax(logits, axis=-1)
        o = jnp.einsum("bhsw,bhswd->bhsd", attn, vg)
        return (lambda x, *d: x.transpose(*d))(o, 0, 2, 1, 3).reshape(B, S, D) @ wo

    x = A_q
    g = _sigmoid((x * gate_w).sum(-1, keepdims=True))
    a = _A_ref(x, A_k, A_v, A_shift_k, A_ssm_k, A_ssm_D)
    b = _B_ref(x, B_wqkv, B_wo)
    return g * a + (1 - g) * b
```

```python
import math

import jax
import jax.numpy as jnp
import numpy as np
from jax.experimental import pallas as pl
from jax.experimental.pallas import tpu as pltpu

S = 2048
D = 640
H = 32
DH = D // H
WIN = 8
DIL = 2
KS = 4
LANES = 128
NT = D // LANES
NA = 32
NB = 64
HALO = 16
KHALO = 8
TM = 256
NI = S // TM


def _neg(a):
    return (a[0], -a[1])


def _add(a, b):
    if a[1] == b[1]:
        return (a[0] + b[0], a[1])
    if a[1] > 0:
        return (a[0] - b[0], 1)
    return (b[0] - a[0], 1)


def _sub(a, b):
    return _add(a, _neg(b))


def _scale(a, c):
    return (a[0] * float(abs(c)), a[1] * (1 if c > 0 else -1))


def _cadd(x, y):
    return (_add(x[0], y[0]), _add(x[1], y[1]))


def _csub(x, y):
    return (_sub(x[0], y[0]), _sub(x[1], y[1]))


def _cmul_i(x, s):
    return (_neg(x[1]), x[0]) if s > 0 else (x[1], _neg(x[0]))


def _ctwiddle(x, num, den):
    num %= den
    if (4 * num) % den == 0:
        for _ in range(4 * num // den):
            x = _cmul_i(x, 1)
        return x
    c, s = math.cos(2 * math.pi * num / den), math.sin(2 * math.pi * num / den)
    re, im = x
    if (8 * num) % den == 0:
        sc, ss = (1 if c > 0 else -1), (1 if s > 0 else -1)
        pick = lambda v, sg: v if sg > 0 else _neg(v)
        return (_scale(_sub(pick(re, sc), pick(im, ss)), abs(c)),
                _scale(_add(pick(re, ss), pick(im, sc)), abs(c)))
    return (_sub(_scale(re, c), _scale(im, s)), _add(_scale(re, s), _scale(im, c)))


def _cfft(z, sgn):
    n = len(z)
    if n == 1:
        return z
    if n == 2:
        return [_cadd(z[0], z[1]), _csub(z[0], z[1])]
    ev = _cfft(z[0::2], sgn)
    o1 = _cfft(z[1::4], sgn)
    o3 = _cfft(z[3::4], sgn)
    out = [None] * n
    for r in range(n // 4):
        t1 = _ctwiddle(o1[r], sgn * r, n)
        t3 = _ctwiddle(o3[r], sgn * 3 * r, n)
        p, m = _cadd(t1, t3), _cmul_i(_csub(t1, t3), sgn)
        out[r], out[r + n // 2] = _cadd(ev[r], p), _csub(ev[r], p)
        out[r + n // 4], out[r + 3 * n // 4] = _cadd(ev[r + n // 4], m), _csub(ev[r + n // 4], m)
    return out


def _odd_fwd(d):
    m = len(d)
    z = [_ctwiddle((d[a], _neg(d[a + m // 2])), -a, 2 * m) for a in range(m // 2)]
    return _cfft(z, -1)


def _odd_bwd(y):
    m = 2 * len(y)
    z = [_ctwiddle(v, a, 2 * m) for a, v in enumerate(_cfft(y, 1))]
    return [v[0] for v in z] + [_neg(v[1]) for v in z]


def _even_fwd(u):
    n = len(u)
    if n == 2:
        return [(u[0], u[1])]
    lo, hi = u[:n // 2], u[n // 2:]
    return (_odd_fwd([_sub(a, b) for a, b in zip(lo, hi)])
            + _even_fwd([_add(a, b) for a, b in zip(lo, hi)]))


def _even_bwd(y):
    n = 2 * len(y)
    if n == 2:
        return [y[0][0], y[0][1]]
    d, s = _odd_bwd(y[:n // 4]), _even_bwd(y[n // 4:])
    return [_add(a, b) for a, b in zip(s, d)] + [_sub(a, b) for a, b in zip(s, d)]


def _block_freqs():
    freqs = [4 * r + 1 for r in range(NA // 2)]
    n = NA
    while n > 2:
        freqs += [(4 * r + 1) * (2 * NA // n) for r in range(n // 4)]
        n //= 2
    return freqs + [None]


def _dft_matrices():
    probe = [(np.ones(()), 1) for _ in range(NA)]
    signs = [(re[1], im[1]) for re, im in _odd_fwd(probe) + _even_fwd(probe)]
    n = 2 * S
    b = np.arange(NB)
    k2 = np.arange(NB)[:, None]
    fwd = np.zeros((NA, 2 * NB, 2, NB))
    inv = np.zeros((NA, 2 * NB, 2, NB))
    for j, f in enumerate(_block_freqs()):
        weight = np.full((2 * NB, 1), 2.0 / n)
        if f is None:
            for part in range(2):
                ang = -2 * np.pi * ((k2 * (b + NB * part)) % (2 * NB)) / (2 * NB)
                fwd[j, :NB, part], fwd[j, NB:, part] = np.cos(ang), np.sin(ang)
                fwd[j, NB, part] = 1.0 - 2.0 * (b % 2)
            weight[0] = weight[NB] = 1.0 / n
        else:
            ang = -2 * np.pi * ((b * (f + 2 * NA * k2)) % n) / n
            fwd[j, :NB, 0], fwd[j, :NB, 1] = np.cos(ang), -np.sin(ang)
            fwd[j, NB:, 0], fwd[j, NB:, 1] = np.sin(ang), np.cos(ang)
        inv[j] = fwd[j] * weight[:, :, None]
        fwd[j] *= np.asarray(signs[j], np.float64)[None, :, None]
    order = lambda g: g.reshape(NA, 2 * NB, 2, NB // 8, 8).transpose(0, 1, 3, 2, 4).reshape(
        NA, 2 * NB, 2 * NB)
    return (order(fwd).astype(jnp.bfloat16),
            order(inv).transpose(0, 2, 1).astype(jnp.bfloat16))


def _value(a):
    return a[0] if a[1] > 0 else -a[0]


def _tile(c):
    return slice(c * LANES, (c + 1) * LANES)


def _kernel(x_hbm, ak_hbm, av_hbm, shift_ref, ssmk_hbm, d_ref, wqkv_hbm, wo_hbm, gw_ref,
            gf_hbm, gi_hbm, out_hbm,
            x_v, ak_v, av_v, ssmk_v, w_v, wp_v, wo_v, wo32, wop_v, gf_v, gi_v,
            qp, kp, vp, filt, ak32, kv32, res, spec, y32, o_v, g_v, out_v, sem_in, sem_x, sem_out):
    f32, bf16 = jnp.float32, jnp.bfloat16

    def w_copy(p):
        return pltpu.make_async_copy(wqkv_hbm.at[:, pl.ds(p * D, D)], w_v.at[p], sem_in.at[p])

    def x_copy(i):
        rows = pl.ds(i * TM, TM)
        return pltpu.make_async_copy(x_hbm.at[rows], x_v.at[rows], sem_x.at[i])

    ssmk_copy = pltpu.make_async_copy(ssmk_hbm, ssmk_v, sem_in.at[3])
    ak_copy = pltpu.make_async_copy(ak_hbm, ak_v, sem_in.at[4])
    av_copy = pltpu.make_async_copy(av_hbm, av_v, sem_in.at[5])
    gf_copy = pltpu.make_async_copy(gf_hbm, gf_v, sem_in.at[6])
    gi_copy = pltpu.make_async_copy(gi_hbm, gi_v, sem_in.at[7])
    wo_copy = pltpu.make_async_copy(wo_hbm, wo_v, sem_in.at[8])

    def out_copy(c):
        return pltpu.make_async_copy(out_v.at[c], out_hbm.at[:, _tile(c)], sem_out.at[c])

    w_copy(1).start()
    for i in range(NI):
        x_copy(i).start()
    for cp in (w_copy(2), ssmk_copy, w_copy(0), ak_copy, av_copy, gf_copy, gi_copy, wo_copy):
        cp.start()

    def permute_columns(p, r0, nrows):
        rows = pl.ds(r0, nrows)
        src = [pltpu.bitcast(w_v[p, rows, _tile(u)], jnp.uint32) for u in range(NT)]
        lane = jax.lax.broadcasted_iota(jnp.int32, src[0].shape, 1)
        for t in range(NT):
            col = (lane % H) * DH + (LANES // H) * t + lane // H
            idx, tile = col % LANES, col // LANES
            acc = jnp.take_along_axis(src[0], idx, axis=1)
            for u in range(1, NT):
                acc = jnp.where(tile == u, jnp.take_along_axis(src[u], idx, axis=1), acc)
            wp_v[p, rows, _tile(t)] = pltpu.bitcast(acc, bf16)

    def project(p, i, dst, halo):
        r0 = pl.multiple_of(i * TM, TM)
        r = jnp.dot(x_v[pl.ds(r0, TM), :], wp_v[p], preferred_element_type=f32)
        for c in range(NT):
            dst[c, pl.ds(halo + r0, TM), :] = r[:, _tile(c)]

    def first_stage(load, beta, lane0):
        r0 = pl.multiple_of(beta * 16, 16)
        for half, fn in enumerate((_odd_fwd, _even_fwd)):
            for j, (re, im) in enumerate(fn([(load(a, half), 1) for a in range(NA)])):
                res[half * (NA // 2) + j, pl.ds(r0, 16), pl.ds(lane0, LANES)] = (
                    jnp.concatenate([re[0], im[0]], axis=0).astype(bf16))

    w_copy(1).wait()
    permute_columns(1, 0, D)
    gate_w = gw_ref[...].astype(f32)

    def k_step(i, carry):
        x_copy(i).wait()
        project(1, i, kp, HALO)
        rows = pl.ds(pl.multiple_of(i * TM, TM), TM)
        z = jnp.sum(x_v[rows, :].astype(f32) * gate_w, axis=-1, keepdims=True)
        g_v[rows, :] = jnp.broadcast_to(1.0 / (1.0 + jnp.exp(-z)), (TM, LANES))
        return carry

    jax.lax.fori_loop(0, NI, k_step, 0)

    w_copy(2).wait()
    permute_columns(2, 0, D)
    ssmk_copy.wait()
    for c in range(NT):
        for t in range(S // 256):
            filt[c, t * 256:(t + 1) * 256, :] = ssmk_v[_tile(c), t * 256:(t + 1) * 256].astype(f32).T

    def v_step(i, carry):
        project(2, i, vp, HALO)
        for c in range(NT):
            first_stage(lambda a, half: filt[c, pl.ds(pl.multiple_of(a * NB + i * 8, 8), 8), :],
                        i, D + c * LANES)
        return carry

    jax.lax.fori_loop(0, NI, v_step, 0)

    w_copy(0).wait()
    permute_columns(0, 0, D)
    ak_copy.wait()
    av_copy.wait()
    for c in range(NT):
        kp[c, 0:HALO, :] = jnp.broadcast_to(kp[c, HALO:HALO + 1, :], (HALO, LANES))
        vp[c, 0:HALO, :] = jnp.broadcast_to(vp[c, HALO:HALO + 1, :], (HALO, LANES))
        ak32[c, 0:KHALO, :] = jnp.zeros((KHALO, LANES), f32)

    def widen(i, carry):
        r0 = pl.multiple_of(i * TM, TM)
        for c in range(NT):
            ak32[c, pl.ds(KHALO + r0, TM), :] = ak_v[pl.ds(r0, TM), _tile(c)].astype(f32)
            kv32[c, pl.ds(r0, TM), :] = av_v[pl.ds(r0, TM), _tile(c)].astype(f32)
        return carry

    jax.lax.fori_loop(0, NI, widen, 0)
    taps = shift_ref[...].astype(f32).T

    def q_step(i, carry):
        project(0, i, qp, 0)
        for c in range(NT):
            tap = [jnp.broadcast_to(taps[t:t + 1, _tile(c)], (8, LANES)) for t in range(KS)]

            def load(a, half):
                r0 = pl.multiple_of(a * NB + i * 8, 8)
                if half == 1:
                    return kv32[c, pl.ds(r0, 8), :]
                acc = ak32[c, pl.ds(KHALO + r0, 8), :] * tap[0]
                for t in range(1, KS):
                    acc = acc + ak32[c, pl.ds(KHALO + r0 - t, 8), :] * tap[t]
                kv = acc * kv32[c, pl.ds(r0, 8), :]
                kv32[c, pl.ds(r0, 8), :] = kv
                return kv

            first_stage(load, i, c * LANES)
        return carry

    jax.lax.fori_loop(0, NI, q_step, 0)

    gf_copy.wait()
    gi_copy.wait()
    wo_copy.wait()
    for c in range(NT):
        wo32[c] = wo_v[:, _tile(c)].astype(f32)
        for dh in range(DH):
            wop_v[dh * H:(dh + 1) * H, _tile(c)] = wo32[c, pl.ds(dh, H, stride=DH), :].astype(bf16)

    exp_scale = DH ** -0.5
    sub = 32

    def attention(r0, masked):
        q = [qp[c, pl.ds(r0, sub), :] for c in range(NT)]
        logits = []
        for w in range(WIN):
            rows = pl.ds(HALO + r0 - DIL * w, sub)
            acc = q[0] * kp[0, rows, :]
            for c in range(1, NT):
                acc = acc + q[c] * kp[c, rows, :]
            acc = acc + pltpu.roll(acc, 2 * H, 1)
            acc = (acc + pltpu.roll(acc, H, 1)) * exp_scale
            if masked and w > 0:
                pos = r0 + jax.lax.broadcasted_iota(jnp.int32, (sub, LANES), 0)
                acc = jnp.where(pos >= DIL * w, acc, -1e9)
            logits.append(acc)
        top = logits[0]
        for w in range(1, WIN):
            top = jnp.maximum(top, logits[w])
        p = [jnp.exp(l - top) for l in logits]
        den = p[0]
        for w in range(1, WIN):
            den = den + p[w]
        norm = (1.0 - g_v[pl.ds(r0, sub), :]) / den
        for c in range(NT):
            acc = p[0] * vp[c, pl.ds(HALO + r0, sub), :]
            for w in range(1, WIN):
                acc = acc + p[w] * vp[c, pl.ds(HALO + r0 - DIL * w, sub), :]
            o_v[pl.ds(r0, sub), _tile(c)] = (acc * norm).astype(bf16)

    def spectrum(j):
        f = jnp.dot(gf_v[j], res[j], preferred_element_type=f32)
        ur, ui, kr, ki = f[:NB, :D], f[NB:, :D], f[:NB, D:], f[NB:, D:]
        rr, ii = ur * kr, ui * ki
        pr, pi = rr - ii, ur * ki + ui * kr
        real = (jax.lax.broadcasted_iota(jnp.int32, (8, D), 0) == 0) & (j == NA - 1)
        pr = jnp.concatenate([jnp.where(real, rr[:8], pr[:8]), pr[8:]], axis=0)
        pi = jnp.concatenate([jnp.where(real, ii[:8], pi[:8]), pi[8:]], axis=0)
        prod = jnp.concatenate([pr, pi], axis=0).astype(bf16)
        back = jnp.dot(gi_v[j], prod, preferred_element_type=f32)
        for c in range(NT):
            spec[c, j] = back[:, _tile(c)]

    def m_step(i, masked):
        for n in range(NA // NI):
            spectrum(i * (NA // NI) + n)
            for m in range(TM // sub // (NA // NI)):
                blk = n * (TM // sub // (NA // NI)) + m
                attention(pl.multiple_of(i * TM + blk * sub, sub), masked and blk == 0)

    m_step(0, True)
    jax.lax.fori_loop(1, NI, lambda i, carry: (m_step(i, False), carry)[1], 0)

    skip = d_ref[...].astype(f32)
    for c in range(NT):
        def column(beta, carry):
            r0 = pl.multiple_of(beta * 16, 16)
            blocks = [((spec[c, j, pl.ds(r0, 8), :], 1), (spec[c, j, pl.ds(r0 + 8, 8), :], 1))
                      for j in range(NA)]
            odd, even = _odd_bwd(blocks[:NA // 2]), _even_bwd(blocks[NA // 2:])
            for a in range(NA):
                y32[pl.ds(pl.multiple_of(a * NB + beta * 8, 8), 8), :] = _value(_add(even[a], odd[a]))
            return carry

        jax.lax.fori_loop(0, NB // 8, column, 0)

        def mix(i, carry):
            rows = pl.ds(pl.multiple_of(i * TM, TM), TM)
            b = jnp.dot(o_v[rows, :], wop_v[:, _tile(c)], preferred_element_type=f32)
            y = y32[rows, :] + kv32[c, rows, :] * skip[:, _tile(c)]
            a = x_v[rows, _tile(c)].astype(f32) * y
            out_v[c, rows, :] = (g_v[rows, :] * a + b).astype(bf16)
            return carry

        jax.lax.fori_loop(0, NI, mix, 0)
        out_copy(c).start()
    for c in range(NT):
        out_copy(c).wait()


@jax.jit
def pallas_gated_mix__ssm_conv_h3__sliding_local_dilated__prompt_kernel(
    A_q: jax.Array,
    A_k: jax.Array,
    A_v: jax.Array,
    A_shift_k: jax.Array,
    A_ssm_k: jax.Array,
    A_ssm_D: jax.Array,
    B_x: jax.Array,
    B_wqkv: jax.Array,
    B_wo: jax.Array,
    gate_w: jax.Array,
):
    del B_x
    assert A_q.shape == (1, S, D) and A_shift_k.shape == (D, KS)
    f32, bf16 = jnp.float32, jnp.bfloat16
    gf, gi = _dft_matrices()
    hbm = pl.BlockSpec(memory_space=pl.ANY)
    vmem = pl.BlockSpec(memory_space=pltpu.VMEM)
    out = pl.pallas_call(
        _kernel,
        out_shape=jax.ShapeDtypeStruct((S, D), bf16),
        in_specs=[hbm, hbm, hbm, vmem, hbm, vmem, hbm, hbm, vmem, hbm, hbm],
        out_specs=hbm,
        scratch_shapes=[
            pltpu.VMEM((S, D), bf16),
            pltpu.VMEM((S, D), bf16),
            pltpu.VMEM((S, D), bf16),
            pltpu.VMEM((D, S), bf16),
            pltpu.VMEM((3, D, D), bf16),
            pltpu.VMEM((3, D, D), bf16),
            pltpu.VMEM((D, D), bf16),
            pltpu.VMEM((NT, D, LANES), f32),
            pltpu.VMEM((D, D), bf16),
            pltpu.VMEM((NA, 2 * NB, 2 * NB), bf16),
            pltpu.VMEM((NA, 2 * NB, 2 * NB), bf16),
            pltpu.VMEM((NT, S, LANES), f32),
            pltpu.VMEM((NT, HALO + S, LANES), f32),
            pltpu.VMEM((NT, HALO + S, LANES), f32),
            pltpu.VMEM((NT, S, LANES), f32),
            pltpu.VMEM((NT, KHALO + S, LANES), f32),
            pltpu.VMEM((NT, S, LANES), f32),
            pltpu.VMEM((NA, 2 * NB, 2 * D), bf16),
            pltpu.VMEM((NT, NA, 2 * NB, LANES), f32),
            pltpu.VMEM((S, LANES), f32),
            pltpu.VMEM((S, D), bf16),
            pltpu.VMEM((S, LANES), f32),
            pltpu.VMEM((NT, S, LANES), bf16),
            pltpu.SemaphoreType.DMA((9,)),
            pltpu.SemaphoreType.DMA((NI,)),
            pltpu.SemaphoreType.DMA((NT,)),
        ],
        compiler_params=pltpu.CompilerParams(vmem_limit_bytes=110 * 1024 * 1024),
        name="gated_mix_h3_local_attn",
    )(A_q.reshape(S, D), A_k.reshape(S, D), A_v.reshape(S, D), A_shift_k, A_ssm_k,
      A_ssm_D.reshape(1, D), B_wqkv, B_wo, gate_w.reshape(1, D), gf, gi)
    return out.reshape(1, S, D)
```

```python
import functools
import math

import jax
import jax.numpy as jnp
import numpy as np
from jax.experimental import pallas as pl
from jax.experimental.pallas import tpu as pltpu

S = 2048
D = 640
H = 32
DH = D // H
WIN = 8
DIL = 2
KS = 4
LANES = 128
NT = D // LANES
NA = 32
NB = 64
HALO = 16
TM = 512
NI = S // TM


class _Pacer:
    def __init__(self):
        self.stores, self.done, self.ops, self.rate = [], 0, 0, 0.0

    def start(self, stores, vector_ops):
        self.flush()
        self.stores, self.done, self.ops = list(stores), 0, 0
        self.rate = len(self.stores) / vector_ops

    def tick(self, ops=0):
        self._emit(min(len(self.stores), int(self.ops * self.rate)))
        self.ops += ops

    def flush(self):
        self._emit(len(self.stores))

    def _emit(self, due):
        while self.done < due:
            self.stores[self.done]()
            self.done += 1


def _neg(a):
    return (a[0], -a[1])


def _mul_i(x, s):
    return (_neg(x[1]), x[0]) if s > 0 else (x[1], _neg(x[0]))


class _Fft:
    def __init__(self, pacer, cosine):
        self.pacer = pacer
        self.cosine = cosine

    def add(self, a, b):
        self.pacer.ops += 1
        if a[1] == b[1]:
            return (a[0] + b[0], a[1])
        return (a[0] - b[0], 1) if a[1] > 0 else (b[0] - a[0], 1)

    def sub(self, a, b):
        return self.add(a, _neg(b))

    def mul(self, a, c):
        self.pacer.ops += 1
        return (a[0] * c[0], a[1] * c[1])

    def cadd(self, x, y):
        return (self.add(x[0], y[0]), self.add(x[1], y[1]))

    def csub(self, x, y):
        return (self.sub(x[0], y[0]), self.sub(x[1], y[1]))

    def cos(self, k):
        k = min(k % 64, -k % 64)
        return (self.cosine(k), 1) if k < 16 else (self.cosine(32 - k), -1)

    def twiddle(self, x, num, den):
        k = (num * (64 // den)) % 64
        if k % 16 == 0:
            for _ in range(k // 16):
                x = _mul_i(x, 1)
            return x
        self.pacer.tick()
        re, im = x
        c = self.cos(k)
        if k % 8 == 0:
            sc, ss = c[1], (1 if k < 32 else -1)
            pick = lambda v, sign: v if sign > 0 else _neg(v)
            return (self.mul(self.sub(pick(re, sc), pick(im, ss)), (c[0], 1)),
                    self.mul(self.add(pick(re, ss), pick(im, sc)), (c[0], 1)))
        s = self.cos(k - 16)
        return (self.sub(self.mul(re, c), self.mul(im, s)),
                self.add(self.mul(re, s), self.mul(im, c)))

    def cfft(self, z, sgn):
        n = len(z)
        if n == 1:
            return [z[0]()]
        if n == 2:
            a, b = z[0](), z[1]()
            return [self.cadd(a, b), self.csub(a, b)]
        ev, o1, o3 = self.cfft(z[0::2], sgn), self.cfft(z[1::4], sgn), self.cfft(z[3::4], sgn)
        out = [None] * n
        for r in range(n // 4):
            t1 = self.twiddle(o1[r], sgn * r, n)
            t3 = self.twiddle(o3[r], sgn * 3 * r, n)
            p, m = self.cadd(t1, t3), _mul_i(self.csub(t1, t3), sgn)
            lo, hi = ev[r], ev[r + n // 4]
            out[r], out[r + n // 2] = self.cadd(lo, p), self.csub(lo, p)
            out[r + n // 4], out[r + 3 * n // 4] = self.cadd(hi, m), self.csub(hi, m)
        return out

    def odd_fwd(self, d):
        m = len(d)
        return self.cfft([lambda a=a: self.twiddle((d[a](), _neg(d[a + m // 2]())), -a, 2 * m)
                          for a in range(m // 2)], -1)

    def odd_bwd(self, y):
        m = 2 * len(y)
        z = [self.twiddle(v, a, 2 * m) for a, v in enumerate(self.cfft(y, 1))]
        return [v[0] for v in z] + [_neg(v[1]) for v in z]

    def even_fwd(self, u):
        n = len(u)
        if n == 2:
            return [(u[0](), u[1]())]
        sums = [None] * (n // 2)

        def diff(a):
            lo, hi = u[a](), u[a + n // 2]()
            sums[a] = self.add(lo, hi)
            return self.sub(lo, hi)

        odd = self.odd_fwd([lambda a=a: diff(a) for a in range(n // 2)])
        return odd + self.even_fwd([lambda v=v: v for v in sums])

    def even_bwd(self, y):
        n = 2 * len(y)
        if n == 2:
            return list(y[0]())
        s, d = self.even_bwd(y[n // 4:]), self.odd_bwd(y[:n // 4])
        return [self.add(a, b) for a, b in zip(s, d)] + [self.sub(a, b) for a, b in zip(s, d)]


def _block_freqs():
    freqs = [4 * r + 1 for r in range(NA // 2)]
    n = NA
    while n > 2:
        freqs += [(4 * r + 1) * (2 * NA // n) for r in range(n // 4)]
        n //= 2
    return freqs + [None]


def _dft_matrices():
    fft = _Fft(_Pacer(), lambda k: 1.0)
    probe = [lambda: (1.0, 1)] * NA
    signs = [(re[1], im[1]) for re, im in fft.odd_fwd(probe) + fft.even_fwd(probe)]
    n = 2 * S
    b = np.arange(NB)
    k2 = np.arange(NB)[:, None]
    fwd = np.zeros((NA, 2 * NB, 2, NB))
    inv = np.zeros((NA, 2 * NB, 2, NB))
    for j, f in enumerate(_block_freqs()):
        weight = np.full((2 * NB, 1), 2.0 / n)
        if f is None:
            for part in range(2):
                ang = -2 * np.pi * ((k2 * (b + NB * part)) % (2 * NB)) / (2 * NB)
                fwd[j, :NB, part], fwd[j, NB:, part] = np.cos(ang), np.sin(ang)
                fwd[j, NB, part] = 1.0 - 2.0 * (b % 2)
            weight[0] = weight[NB] = 1.0 / n
        else:
            ang = -2 * np.pi * ((b * (f + 2 * NA * k2)) % n) / n
            fwd[j, :NB, 0], fwd[j, :NB, 1] = np.cos(ang), -np.sin(ang)
            fwd[j, NB:, 0], fwd[j, NB:, 1] = np.sin(ang), np.cos(ang)
        inv[j] = fwd[j] * weight[:, :, None]
        fwd[j] *= np.asarray(signs[j], np.float64)[None, :, None]
    order = lambda g: g.reshape(NA, 2 * NB, 2, NB // 8, 8).transpose(0, 1, 3, 2, 4).reshape(
        NA, 2 * NB, 2 * NB)
    return (order(fwd).astype(jnp.bfloat16),
            order(inv).transpose(0, 2, 1).astype(jnp.bfloat16))


def _value(a):
    return a[0] if a[1] > 0 else -a[0]


_Q, _K, _V, _FILT, _AK, _GATE, _MISC = 0, NT, 2 * NT, 3 * NT, 4 * NT, 5 * NT, 5 * NT + 1
_SPEC = _FILT
_PROJ = _Q
_COS, _TAP, _SKIP, _GW, _DUMMY = 0, 16, 16 + KS * NT, 16 + (KS + 1) * NT, 16 + (KS + 2) * NT
LOG2E = math.log2(math.e)


def _tile(c):
    return slice(c * LANES, (c + 1) * LANES)


def _kernel(x_hbm, ak_hbm, av_hbm, shift_ref, ssmk_hbm, d_ref, wqkv_hbm, wo_hbm, gw_ref,
            gf_hbm, gi_hbm, out_hbm,
            x_v, ak_v, av_v, ssmk_v, w_v, wt_v, wo_v, wop_v, words, gf_v, gi_v,
            buf, kv32, res, y32, o_v, out_v, sem_in, sem_x, sem_out):
    f32, bf16 = jnp.float32, jnp.bfloat16
    pacer = _Pacer()

    def w_copy(p):
        return pltpu.make_async_copy(wqkv_hbm.at[:, pl.ds(p * D, D)], w_v.at[p], sem_in.at[p])

    def x_copy(i):
        rows = pl.ds(i * TM, TM)
        return pltpu.make_async_copy(x_hbm.at[rows], x_v.at[rows], sem_x.at[i])

    ssmk_copy = pltpu.make_async_copy(ssmk_hbm, ssmk_v, sem_in.at[3])
    ak_copy = pltpu.make_async_copy(ak_hbm, ak_v, sem_in.at[4])
    av_copy = pltpu.make_async_copy(av_hbm, av_v, sem_in.at[5])
    gf_copy = pltpu.make_async_copy(gf_hbm, gf_v, sem_in.at[6])
    gi_copy = pltpu.make_async_copy(gi_hbm, gi_v, sem_in.at[7])
    wo_copy = pltpu.make_async_copy(wo_hbm, wo_v, sem_in.at[8])

    def out_copy(i):
        rows = pl.ds(pl.multiple_of(i * 16, 16), 16)
        return pltpu.make_async_copy(out_v.at[i], out_hbm.at[:, rows, :], sem_out.at[i])

    def rows_at(start, size):
        return pl.ds(pl.multiple_of(HALO + start, 8), size)

    def misc(reg, zero):
        return buf[_MISC, pl.ds(pl.multiple_of(zero + reg * 8, 8), 8), :]

    def reorder_rows(tile, dst, u):
        words[u] = pltpu.bitcast(tile, jnp.uint32)
        for pair in range(DH // 2):
            dst[pair * 2 * H:(pair + 1) * 2 * H, _tile(u)] = pltpu.bitcast(
                words[u, pl.ds(pair, H, stride=DH // 2), :], bf16)

    def prepare_weight(p):
        for u in range(NT):
            reorder_rows(w_v[p, _tile(u), :].T, wt_v.at[p], u)

    def result_stores(r, plane, r0, scale=None, group=32):
        def put(c, v):
            val = r[v * group:(v + 1) * group, _tile(c)]
            buf[plane + c, rows_at(r0 + v * group, group), :] = val if scale is None else val * scale
        return [functools.partial(put, c, v) for c in range(NT) for v in range(r.shape[0] // group)]

    def project(p, r0):
        return jax.lax.dot_general(x_v[pl.ds(r0, TM), :], wt_v[p], (((1,), (1,)), ((), ())),
                                   preferred_element_type=f32)

    def first_stage(fft, load, beta, col):
        r0 = pl.multiple_of(beta * 16, 16)
        for half, fn in enumerate((fft.odd_fwd, fft.even_fwd)):
            outs = fn([lambda a=a: (load(a, half), 1) for a in range(NA)])
            for j, (re, im) in enumerate(outs):
                res[half * (NA // 2) + j, pl.ds(r0, 16), _tile(col)] = (
                    jnp.concatenate([re[0], im[0]], axis=0).astype(bf16))

    lane_head = lambda axis: (jax.lax.broadcasted_iota(jnp.int32, (LANES, LANES), axis) % (2 * H)) // 2

    w_copy(1).start()
    x_copy(0).start()
    x_copy(1).start()
    for k in range(1, 16):
        buf[_MISC, (_COS + k) * 8:(_COS + k + 1) * 8, :] = jnp.full(
            (8, LANES), math.cos(2 * math.pi * k / 64), f32)
    taps = shift_ref[...].astype(f32).T
    skip, gate_w = d_ref[...].astype(f32), gw_ref[...].astype(f32)
    for c in range(NT):
        rows = [taps[t:t + 1] for t in range(KS)] + [skip, gate_w]
        for n, row in enumerate(rows):
            reg = _TAP + n * NT + c
            buf[_MISC, reg * 8:(reg + 1) * 8, :] = jnp.broadcast_to(row[:, _tile(c)], (8, LANES))
        buf[_AK + c, 0:HALO, :] = jnp.zeros((HALO, LANES), f32)
    w_copy(1).wait()
    prepare_weight(1)

    def k_step(i, widen):
        r0 = pl.multiple_of(i * TM, TM)
        zero = (i // NI) * 8
        pacer.start(result_stores(project(1, r0), _K, r0), (TM // 16) * (30 + 40 * widen) * 1.1)
        parts = []
        for v in range(TM // 16):
            pacer.tick(30)
            xs = x_v[pl.ds(r0 + v * 16, 16), :].astype(f32)
            acc = None
            for c in range(NT):
                gw = misc(_GW + c, zero)
                term = xs[:, _tile(c)] * jnp.concatenate([gw, gw], axis=0)
                acc = term if acc is None else acc + term
            parts.append(acc.astype(bf16))
            if widen:
                pacer.tick(40)
                for n in range(NI):
                    rows = (v * NI + n) * 16
                    wide = ak_v[rows:rows + 16, :].astype(f32)
                    for c in range(NT):
                        buf[_AK + c, rows_at(zero + rows, 16), :] = wide[:, _tile(c)]
        pacer.flush()
        z = jnp.dot(jnp.concatenate(parts, axis=0), jnp.ones((LANES, LANES), bf16),
                    preferred_element_type=f32)
        buf[_GATE, rows_at(r0, TM), :] = 1.0 / (1.0 + jnp.exp(-z))

    def k_loop(i, carry):
        x_copy(i).wait()

        @pl.when(i == 0)
        def _():
            for cp in (x_copy(2), x_copy(3), ak_copy):
                cp.start()

        @pl.when(i == 1)
        def _():
            for cp in (w_copy(2), ssmk_copy):
                cp.start()

        k_step(i, False)
        return carry

    jax.lax.fori_loop(0, NI - 1, k_loop, 0)
    w_copy(0).start()
    av_copy.start()
    x_copy(NI - 1).wait()
    ak_copy.wait()
    jax.lax.fori_loop(NI - 1, NI, lambda i, carry: (k_step(i, True), carry)[1], 0)

    w_copy(2).wait()
    prepare_weight(2)
    ssmk_copy.wait()
    for cp in (gf_copy, gi_copy, wo_copy):
        cp.start()
    for c in range(NT):
        for t in range(S // 256):
            buf[_FILT + c, HALO + t * 256:HALO + (t + 1) * 256, :] = (
                ssmk_v[_tile(c), t * 256:(t + 1) * 256].astype(f32).T)

    def v_step(i, carry):
        r0 = pl.multiple_of(i * TM, TM)
        zero = (i // NI) * 8
        fft = _Fft(pacer, lambda k: misc(_COS + k, zero))
        pacer.start(result_stores(project(2, r0), _V, r0), 2 * NT * 452 * 1.08)
        for c in range(NT):
            for h in range(2):
                def load(a, half):
                    pacer.tick()
                    return buf[_FILT + c, rows_at(a * NB + i * 16 + h * 8, 8), :]

                first_stage(fft, load, 2 * i + h, 2 * c + 1)
        pacer.flush()
        return carry

    jax.lax.fori_loop(0, NI, v_step, 0)

    w_copy(0).wait()
    prepare_weight(0)
    av_copy.wait()
    for c in range(NT):
        for plane in (_K, _V):
            buf[plane + c, 0:HALO, :] = jnp.broadcast_to(buf[plane + c, HALO:HALO + 1, :], (HALO, LANES))

    def q_step(i, carry):
        r0 = pl.multiple_of(i * TM, TM)
        zero = (i // NI) * 8
        fft = _Fft(pacer, lambda k: misc(_COS + k, zero))
        pacer.start(result_stores(project(0, r0), _Q, r0, scale=DH ** -0.5 * LOG2E),
                    2 * NT * (452 + 9 * NA) * 1.06)
        for c in range(NT):
            for h in range(2):
                def load(a, half):
                    row = a * NB + i * 16
                    dst = pl.ds(pl.multiple_of(row + h * 8, 8), 8)
                    if half == 1:
                        return kv32[c, dst, :]
                    pacer.tick(9)
                    acc = None
                    for t in range(KS):
                        term = (buf[_AK + c, pl.ds(HALO + row + h * 8 - t, 8), :]
                                * misc(_TAP + t * NT + c, zero))
                        acc = term if acc is None else acc + term
                    v = av_v[pl.ds(pl.multiple_of(row, 16), 16), _tile(c)].astype(f32)
                    kv = acc * v[h * 8:(h + 1) * 8]
                    kv32[c, dst, :] = kv
                    return kv

                first_stage(fft, load, 2 * i + h, 2 * c)
        pacer.flush()
        return carry

    jax.lax.fori_loop(0, NI, q_step, 0)

    gf_copy.wait()
    gi_copy.wait()
    wo_copy.wait()
    for u in range(NT):
        reorder_rows(wo_v[:, _tile(u)], wop_v, u)

    steps = NA // NI

    def m_step(i, first):
        zero = (i // NI) * 8
        same_head = (lane_head(0) == lane_head(1)).astype(bf16)

        def forward(n):
            f = jnp.dot(gf_v[i * steps + n], res[i * steps + n], preferred_element_type=f32)

            def mark(c, v):
                buf[_MISC, pl.ds(pl.multiple_of(zero + _DUMMY * 8, 8), 8), :] = (
                    f[v * 32:v * 32 + 8, _tile(c)])
            return f, [functools.partial(mark, c, v) for c in range(0, 2 * NT, 4) for v in range(4)]

        def product(f, n):
            cols = []
            for c in range(NT):
                u, k = f[:, _tile(2 * c)], f[:, _tile(2 * c + 1)]
                ur, ui, kr, ki = u[:NB], u[NB:], k[:NB], k[NB:]
                rr, ii = ur * kr, ui * ki
                pr, pi = rr - ii, ur * ki + ui * kr
                if n == steps - 1:
                    real = (jax.lax.broadcasted_iota(jnp.int32, (8, LANES), 0) == 0) & (i == NI - 1)
                    pr = jnp.concatenate([jnp.where(real, rr[:8], pr[:8]), pr[8:]], axis=0)
                    pi = jnp.concatenate([jnp.where(real, ii[:8], pi[:8]), pi[8:]], axis=0)
                cols.append(jnp.concatenate([pr, pi], axis=0).astype(bf16))
            return jnp.concatenate(cols, axis=1)

        def inverse(prod, n):
            back = jnp.dot(gi_v[i * steps + n], prod, preferred_element_type=f32)
            j = i * steps + n
            return result_stores(back, _SPEC + NT * (j // (NA // 2)), (j % (NA // 2)) * 2 * NB)

        def scores(n):
            parts = []
            for v in range(4):
                r0 = i * TM + n * NB + v * 16
                q = [buf[_Q + c, rows_at(r0, 16), :] for c in range(NT)]
                for w in range(WIN):
                    pacer.tick(19)
                    acc = None
                    for c in range(NT):
                        term = q[c] * buf[_K + c, pl.ds(HALO + r0 - DIL * w, 16), :]
                        acc = term if acc is None else acc + term
                    parts.append(acc.astype(bf16))
            return jnp.concatenate(parts, axis=0)

        def attend(logits, n, v):
            r0 = i * TM + n * NB + v * 16
            lg = [logits[(v * WIN + w) * 16:(v * WIN + w + 1) * 16] for w in range(WIN)]
            if first and n == 0 and v == 0:
                pos = r0 + jax.lax.broadcasted_iota(jnp.int32, (16, LANES), 0)
                lg = [jnp.where(pos >= DIL * w, l, -1e9 * LOG2E) for w, l in enumerate(lg)]
            top = functools.reduce(jnp.maximum, lg)
            p = [jnp.exp2(l - top) for l in lg]
            pacer.tick(52)
            norm = (1.0 - buf[_GATE, rows_at(r0, 16), :]) / functools.reduce(jnp.add, p)
            for c in range(NT):
                pacer.tick(33)
                acc = None
                for w in range(WIN):
                    term = p[w] * buf[_V + c, pl.ds(HALO + r0 - DIL * w, 16), :]
                    acc = term if acc is None else acc + term
                o_v[v, pl.ds(pl.multiple_of((i * steps + n) * 16, 16), 16), _tile(c)] = (
                    (acc * norm).astype(bf16))

        score_ops, attend_ops = 4 * WIN * 19, 52 + NT * 33
        f, marks = forward(0)
        pacer.start(marks, score_ops)
        part = scores(0)
        late = []
        for n in range(steps):
            prod = product(f, n)
            if n + 1 < steps:
                f, marks = forward(n + 1)
                pacer.start(marks, score_ops + len(late) * attend_ops)
            for fn in late:
                fn()
            logits = jnp.dot(part, same_head, preferred_element_type=f32)
            if n + 1 < steps:
                part = scores(n + 1)
            early = 2 if n + 1 < steps else 4
            pacer.start(inverse(prod, n), early * attend_ops)
            for v in range(early):
                attend(logits, n, v)
            late = [functools.partial(attend, logits, n, v) for v in range(early, 4)]
        pacer.flush()

    jax.lax.fori_loop(0, NI, lambda i, carry: (m_step(i, True), carry)[1], 0)

    def w_step(i, carry):
        zero = (i // NI) * 8
        fft = _Fft(pacer, lambda k: misc(_COS + k, zero))
        proj = jnp.dot(o_v[i], wop_v[...], preferred_element_type=f32)
        pacer.start(result_stores(proj, _PROJ, zero), NT * 2 * 484 + (NT - 1) * NA * 13)

        def mix(c):
            skip_c = misc(_SKIP + c, zero)
            skip_c = jnp.concatenate([skip_c, skip_c], axis=0)
            for a in range(NA):
                pacer.tick(13)
                row = pl.multiple_of(a * NB + i * 16, 16)
                y = y32[c, a * 16:(a + 1) * 16, :] + kv32[c, pl.ds(row, 16), :] * skip_c
                gated = buf[_GATE, rows_at(row, 16), :] * x_v[pl.ds(row, 16), _tile(c)].astype(f32)
                out_v[i, a, :, _tile(c)] = (
                    gated * y + buf[_PROJ + c, rows_at(zero + a * 16, 16), :]).astype(bf16)

        for c in range(NT):
            for h in range(2):
                def load(j):
                    pacer.tick()
                    plane = _SPEC + NT * (j // (NA // 2)) + c
                    row = (j % (NA // 2)) * 2 * NB + (2 * i + h) * 16
                    return ((buf[plane, rows_at(row, 8), :], 1), (buf[plane, rows_at(row + 8, 8), :], 1))

                blocks = [functools.partial(load, j) for j in range(NA)]
                even, odd = fft.even_bwd(blocks[NA // 2:]), fft.odd_bwd(blocks[:NA // 2])
                for a in range(NA):
                    y32[c, a * 16 + h * 8:a * 16 + (h + 1) * 8, :] = _value(fft.add(even[a], odd[a]))
            if c > 0:
                mix(c - 1)
        pacer.flush()
        mix(NT - 1)
        out_copy(i).start()
        return carry

    jax.lax.fori_loop(0, NI, w_step, 0)
    for i in range(NI):
        out_copy(i).wait()


@jax.jit
def pallas_gated_mix__ssm_conv_h3__sliding_local_dilated__prompt_kernel(
    A_q: jax.Array,
    A_k: jax.Array,
    A_v: jax.Array,
    A_shift_k: jax.Array,
    A_ssm_k: jax.Array,
    A_ssm_D: jax.Array,
    B_x: jax.Array,
    B_wqkv: jax.Array,
    B_wo: jax.Array,
    gate_w: jax.Array,
):
    del B_x
    assert A_q.shape == (1, S, D) and A_shift_k.shape == (D, KS)
    f32, bf16 = jnp.float32, jnp.bfloat16
    gf, gi = _dft_matrices()
    hbm = pl.BlockSpec(memory_space=pl.ANY)
    vmem = pl.BlockSpec(memory_space=pltpu.VMEM)
    out = pl.pallas_call(
        _kernel,
        out_shape=jax.ShapeDtypeStruct((NA, NB, D), bf16),
        in_specs=[hbm, hbm, hbm, vmem, hbm, vmem, hbm, hbm, vmem, hbm, hbm],
        out_specs=hbm,
        scratch_shapes=[
            pltpu.VMEM((S, D), bf16),
            pltpu.VMEM((S, D), bf16),
            pltpu.VMEM((S, D), bf16),
            pltpu.VMEM((D, S), bf16),
            pltpu.VMEM((3, D, D), bf16),
            pltpu.VMEM((3, D, D), bf16),
            pltpu.VMEM((D, D), bf16),
            pltpu.VMEM((D, D), bf16),
            pltpu.VMEM((NT, D // 2, LANES), jnp.uint32),
            pltpu.VMEM((NA, 2 * NB, 2 * NB), bf16),
            pltpu.VMEM((NA, 2 * NB, 2 * NB), bf16),
            pltpu.VMEM((_MISC + 1, HALO + S, LANES), f32),
            pltpu.VMEM((NT, S, LANES), f32),
            pltpu.VMEM((NA, 2 * NB, 2 * D), bf16),
            pltpu.VMEM((NT, TM, LANES), f32),
            pltpu.VMEM((NI, TM, D), bf16),
            pltpu.VMEM((NI, NA, 16, D), bf16),
            pltpu.SemaphoreType.DMA((9,)),
            pltpu.SemaphoreType.DMA((NI,)),
            pltpu.SemaphoreType.DMA((NI,)),
        ],
        compiler_params=pltpu.CompilerParams(vmem_limit_bytes=110 * 1024 * 1024),
        name="gated_mix_h3_local_attn",
    )(A_q.reshape(S, D), A_k.reshape(S, D), A_v.reshape(S, D), A_shift_k, A_ssm_k,
      A_ssm_D.reshape(1, D), B_wqkv, B_wo, gate_w.reshape(1, D), gf, gi)
    return out.reshape(1, S, D)
```

```python
import functools
import math

import jax
import jax.numpy as jnp
import numpy as np
from jax.experimental import pallas as pl
from jax.experimental.pallas import tpu as pltpu

S = 2048
D = 640
H = 32
DH = D // H
WIN = 8
DIL = 2
KS = 4
LANES = 128
NT = D // LANES
NA = 32
NB = 64
HALO = 16
TM = 512
NI = S // TM


class _Pacer:
    def __init__(self):
        self.stores, self.done, self.ops, self.rate = [], 0, 0, 0.0

    def start(self, stores, vector_ops):
        self.flush()
        self.stores, self.done, self.ops = list(stores), 0, 0
        self.rate = len(self.stores) / vector_ops

    def tick(self, ops=0):
        self.emit(min(len(self.stores), int(self.ops * self.rate)))
        self.ops += ops

    def flush(self):
        self.emit(len(self.stores))

    def emit(self, due):
        while self.done < due:
            self.stores[self.done]()
            self.done += 1


def _neg(a):
    return (a[0], -a[1])


def _mul_i(x, s):
    return (_neg(x[1]), x[0]) if s > 0 else (x[1], _neg(x[0]))


class _Fft:
    def __init__(self, pacer, cosine):
        self.pacer = pacer
        self.cosine = cosine

    def add(self, a, b):
        self.pacer.ops += 1
        if a[1] == b[1]:
            return (a[0] + b[0], a[1])
        return (a[0] - b[0], 1) if a[1] > 0 else (b[0] - a[0], 1)

    def sub(self, a, b):
        return self.add(a, _neg(b))

    def mul(self, a, c):
        self.pacer.ops += 1
        return (a[0] * c[0], a[1] * c[1])

    def cadd(self, x, y):
        return (self.add(x[0], y[0]), self.add(x[1], y[1]))

    def csub(self, x, y):
        return (self.sub(x[0], y[0]), self.sub(x[1], y[1]))

    def cos(self, k):
        k = min(k % 64, -k % 64)
        return (self.cosine(k), 1) if k < 16 else (self.cosine(32 - k), -1)

    def twiddle(self, x, num, den):
        k = (num * (64 // den)) % 64
        if k % 16 == 0:
            for _ in range(k // 16):
                x = _mul_i(x, 1)
            return x
        self.pacer.tick()
        re, im = x
        c = self.cos(k)
        if k % 8 == 0:
            sc, ss = c[1], (1 if k < 32 else -1)
            pick = lambda v, sign: v if sign > 0 else _neg(v)
            return (self.mul(self.sub(pick(re, sc), pick(im, ss)), (c[0], 1)),
                    self.mul(self.add(pick(re, ss), pick(im, sc)), (c[0], 1)))
        s = self.cos(k - 16)
        return (self.sub(self.mul(re, c), self.mul(im, s)),
                self.add(self.mul(re, s), self.mul(im, c)))

    def cfft(self, z, sgn):
        n = len(z)
        if n == 1:
            return [z[0]()]
        if n == 2:
            a, b = z[0](), z[1]()
            return [self.cadd(a, b), self.csub(a, b)]
        ev, o1, o3 = self.cfft(z[0::2], sgn), self.cfft(z[1::4], sgn), self.cfft(z[3::4], sgn)
        out = [None] * n
        for r in range(n // 4):
            t1 = self.twiddle(o1[r], sgn * r, n)
            t3 = self.twiddle(o3[r], sgn * 3 * r, n)
            p, m = self.cadd(t1, t3), _mul_i(self.csub(t1, t3), sgn)
            lo, hi = ev[r], ev[r + n // 4]
            out[r], out[r + n // 2] = self.cadd(lo, p), self.csub(lo, p)
            out[r + n // 4], out[r + 3 * n // 4] = self.cadd(hi, m), self.csub(hi, m)
        return out

    def odd_fwd(self, d):
        m = len(d)
        return self.cfft([lambda a=a: self.twiddle((d[a](), _neg(d[a + m // 2]())), -a, 2 * m)
                          for a in range(m // 2)], -1)

    def odd_bwd(self, y):
        m = 2 * len(y)
        z = [self.twiddle(v, a, 2 * m) for a, v in enumerate(self.cfft(y, 1))]
        return [v[0] for v in z] + [_neg(v[1]) for v in z]

    def even_fwd(self, u):
        n = len(u)
        if n == 2:
            return [(u[0](), u[1]())]
        sums = [None] * (n // 2)

        def diff(a):
            lo, hi = u[a](), u[a + n // 2]()
            sums[a] = self.add(lo, hi)
            return self.sub(lo, hi)

        odd = self.odd_fwd([lambda a=a: diff(a) for a in range(n // 2)])
        return odd + self.even_fwd([lambda v=v: v for v in sums])

    def even_bwd(self, y):
        n = 2 * len(y)
        if n == 2:
            return list(y[0]())
        s, d = self.even_bwd(y[n // 4:]), self.odd_bwd(y[:n // 4])
        return [self.add(a, b) for a, b in zip(s, d)] + [self.sub(a, b) for a, b in zip(s, d)]


def _block_freqs():
    freqs = [4 * r + 1 for r in range(NA // 2)]
    n = NA
    while n > 2:
        freqs += [(4 * r + 1) * (2 * NA // n) for r in range(n // 4)]
        n //= 2
    return freqs + [None]


def _dft_matrices():
    fft = _Fft(_Pacer(), lambda k: 1.0)
    probe = [lambda: (1.0, 1)] * NA
    signs = [(re[1], im[1]) for re, im in fft.odd_fwd(probe) + fft.even_fwd(probe)]
    n = 2 * S
    b = np.arange(NB)
    k2 = np.arange(NB)[:, None]
    fwd = np.zeros((NA, 2 * NB, 2, NB))
    inv = np.zeros((NA, 2 * NB, 2, NB))
    for j, f in enumerate(_block_freqs()):
        weight = np.full((2 * NB, 1), 2.0 / n)
        if f is None:
            for part in range(2):
                ang = -2 * np.pi * ((k2 * (b + NB * part)) % (2 * NB)) / (2 * NB)
                fwd[j, :NB, part], fwd[j, NB:, part] = np.cos(ang), np.sin(ang)
                fwd[j, NB, part] = 1.0 - 2.0 * (b % 2)
            weight[0] = weight[NB] = 1.0 / n
        else:
            ang = -2 * np.pi * ((b * (f + 2 * NA * k2)) % n) / n
            fwd[j, :NB, 0], fwd[j, :NB, 1] = np.cos(ang), -np.sin(ang)
            fwd[j, NB:, 0], fwd[j, NB:, 1] = np.sin(ang), np.cos(ang)
        inv[j] = fwd[j] * weight[:, :, None]
        fwd[j] *= np.asarray(signs[j], np.float64)[None, :, None]
    order = lambda g: g.reshape(NA, 2, NB // 8, 8, 2, NB // 8, 8).transpose(
        0, 2, 1, 3, 5, 4, 6).reshape(NA, 2 * NB, 2 * NB)
    return (order(fwd).astype(jnp.bfloat16),
            order(inv).transpose(0, 2, 1).astype(jnp.bfloat16))


def _value(a):
    return a[0] if a[1] > 0 else -a[0]


_Q, _K, _V, _FILT, _AK, _KV, _MISC = (n * NT for n in range(7))
_GATE = _MISC + 1
_LOGITS = _MISC + 2
_SPEC = _FILT
_PROJ = _Q
_COS, _TAP, _SKIP, _GW, _DUMMY = 0, 16, 16 + KS * NT, 16 + (KS + 1) * NT, 16 + (KS + 2) * NT
LOG2E = math.log2(math.e)


def _tile(c):
    return slice(c * LANES, (c + 1) * LANES)


def _kernel(x_hbm, ak_hbm, av_hbm, shift_ref, ssmk_hbm, d_ref, wqkv_hbm, wo_hbm, gw_ref,
            gf_hbm, gi_hbm, out_hbm,
            x_v, ak_v, av_v, ssmk_v, w_v, wt_v, wo_v, wop_v, words, gf_v, gi_v,
            buf, gate_v, res, part_v, y32, o_v, out_v, sem_in, sem_x, sem_out):
    f32, bf16 = jnp.float32, jnp.bfloat16
    pacer = _Pacer()

    def w_copy(p):
        return pltpu.make_async_copy(wqkv_hbm.at[:, pl.ds(p * D, D)], w_v.at[p], sem_in.at[p])

    def x_copy(i):
        rows = pl.ds(i * (S // 2), S // 2)
        return pltpu.make_async_copy(x_hbm.at[rows], x_v.at[rows], sem_x.at[i])

    ssmk_copy = pltpu.make_async_copy(ssmk_hbm, ssmk_v, sem_in.at[3])
    ak_copy = pltpu.make_async_copy(ak_hbm, ak_v, sem_in.at[4])
    av_copy = pltpu.make_async_copy(av_hbm, av_v, sem_in.at[5])
    gf_copy = pltpu.make_async_copy(gf_hbm, gf_v, sem_in.at[6])
    gi_copy = pltpu.make_async_copy(gi_hbm, gi_v, sem_in.at[7])
    wo_copy = pltpu.make_async_copy(wo_hbm, wo_v, sem_in.at[8])

    def out_copy(i):
        rows = pl.ds(pl.multiple_of(i * 16, 16), 16)
        return pltpu.make_async_copy(out_v.at[i], out_hbm.at[:, rows, :], sem_out.at[i])

    def rows_at(start, size):
        return pl.ds(pl.multiple_of(HALO + start, 8), size)

    def misc(reg, zero):
        return buf[_MISC, pl.ds(pl.multiple_of(zero + reg * 8, 8), 8), :]

    def reorder_rows(tile, dst, u):
        words[u] = pltpu.bitcast(tile, jnp.uint32)
        for pair in range(DH // 2):
            dst[pair * 2 * H:(pair + 1) * 2 * H, _tile(u)] = pltpu.bitcast(
                words[u, pl.ds(pair, H, stride=DH // 2), :], bf16)

    def prepare_weight(p):
        for u in range(NT):
            reorder_rows(w_v[p, _tile(u), :].T, wt_v.at[p], u)

    def matmul_stores(mm, plane, r0, scale=None):
        k_head, k_tail, quarter = slice(0, D - LANES), slice(D - LANES, D), TM // 4
        staged = mm(slice(0, TM), k_tail, k_head)
        last = [mm(slice(n * quarter, (n + 1) * quarter), k_tail, k_tail) for n in range(4)]
        full = [mm(slice(0, TM), k_head, _tile(c)) for c in range(NT)]

        def stage(v):
            for c in range(NT - 1):
                buf[plane + c, rows_at(r0 + v * 32, 32), :] = staged[v * 32:(v + 1) * 32, _tile(c)]

        def stage_last(v):
            for n in range(4):
                buf[plane + NT - 1, rows_at(r0 + n * quarter + v * 32, 32), :] = (
                    last[n][v * 32:(v + 1) * 32])

        def finish(c, v):
            rows = rows_at(r0 + v * 32, 32)
            val = full[c][v * 32:(v + 1) * 32] + buf[plane + c, rows, :]
            buf[plane + c, rows, :] = val if scale is None else val * scale

        return ([functools.partial(stage, v) for v in range(TM // 32)]
                + [functools.partial(stage_last, v) for v in range(quarter // 32)]
                + [functools.partial(finish, c, v) for c in range(NT) for v in range(TM // 32)])

    lane_head = lambda axis: (jax.lax.broadcasted_iota(jnp.int32, (LANES, LANES), axis) % (2 * H)) // 2

    def gate(i, zero):
        for v in range(TM // 16):
            pacer.tick(30)
            xs = x_v[pl.ds(pl.multiple_of(i * TM + v * 16, 16), 16), :].astype(f32)
            acc = None
            for c in range(NT):
                gw = misc(_GW + c, zero)
                term = xs[:, _tile(c)] * jnp.concatenate([gw, gw], axis=0)
                acc = term if acc is None else acc + term
            gate_v[pl.ds(pl.multiple_of(i * TM + v * 16, 16), 16), :] = acc.astype(bf16)

    def first_stage(plane, col, beta, zero):
        fft = _Fft(pacer, lambda k: misc(_COS + k, zero))
        r0 = pl.multiple_of(beta * 16, 16)
        for c in range(NT):
            def load(a):
                pacer.tick()
                return (buf[plane + c, rows_at(a * NB + beta * 8, 8), :], 1)

            for half, fn in enumerate((fft.odd_fwd, fft.even_fwd)):
                outs = fn([functools.partial(load, a) for a in range(NA)])
                for j, (re, im) in enumerate(outs):
                    res[half * (NA // 2) + j, pl.ds(r0, 16), _tile(2 * c + col)] = (
                        jnp.concatenate([re[0], im[0]], axis=0).astype(bf16))

    def widen_k(r0, zero):
        for v in range(2 * TM // 32):
            pacer.tick(30)
            wide = ak_v[pl.ds(pl.multiple_of(r0 + v * 32, 32), 32), :].astype(f32)
            for c in range(NT):
                buf[_AK + c, rows_at(r0 + v * 32, 32), :] = wide[:, _tile(c)]

    def shift_conv(r0, zero):
        for v in range(2 * TM // 16):
            row = pl.multiple_of(r0 + v * 16, 16)
            vals = av_v[pl.ds(row, 16), :].astype(f32)
            kv = []
            for c in range(NT):
                pacer.tick(19)
                acc = None
                for t in range(KS):
                    tap = misc(_TAP + t * NT + c, zero)
                    term = (buf[_AK + c, pl.ds(HALO + row - t, 16), :]
                            * jnp.concatenate([tap, tap], axis=0))
                    acc = term if acc is None else acc + term
                kv.append(acc * vals[:, _tile(c)])
            for c in range(NT):
                buf[_KV + c, rows_at(row, 16), :] = kv[c]

    def scores(i, n):
        for v in range(4):
            r0 = i * TM + n * NB + v * 16
            q = [buf[_Q + c, rows_at(r0, 16), :] for c in range(NT)]
            for w in range(WIN):
                pacer.tick(19)
                acc = None
                for c in range(NT):
                    term = q[c] * buf[_K + c, pl.ds(HALO + r0 - DIL * w, 16), :]
                    acc = term if acc is None else acc + term
                part_v[i * steps + n, (v * WIN + w) * 16:(v * WIN + w + 1) * 16, :] = acc.astype(bf16)

    gate_ops, stage_ops, score_ops = TM // 16 * 30, NT * 452, 4 * WIN * 19
    steps = NA // NI
    early = steps // 2

    def projection(p, plane, lo, hi, vector_ops, work, scale=None):
        def step(i, carry):
            r0 = pl.multiple_of(i * TM, TM)

            def mm(rows, k, n):
                lhs = x_v[pl.ds(r0 + rows.start, rows.stop - rows.start), k]
                return jax.lax.dot_general(lhs, wt_v[p, n, k], (((1,), (1,)), ((), ())),
                                           preferred_element_type=f32)

            pacer.start(matmul_stores(mm, plane, r0, scale), vector_ops * 1.06)
            work(i, (i // NI) * 8)
            pacer.flush()
            return carry

        jax.lax.fori_loop(lo, hi, step, 0)

    def fill_halo(plane):
        for c in range(NT):
            buf[plane + c, 0:HALO, :] = jnp.broadcast_to(buf[plane + c, HALO:HALO + 1, :], (HALO, LANES))

    for cp in (w_copy(0), x_copy(0)):
        cp.start()
    for k in range(1, 16):
        buf[_MISC, (_COS + k) * 8:(_COS + k + 1) * 8, :] = jnp.full(
            (8, LANES), math.cos(2 * math.pi * k / 64), f32)
    rows = [shift_ref[...].astype(f32)[t:t + 1] for t in range(KS)]
    rows += [d_ref[...].astype(f32).reshape(1, D), gw_ref[...].astype(f32).reshape(1, D)]
    for c in range(NT):
        for n, row in enumerate(rows):
            reg = _TAP + n * NT + c
            buf[_MISC, reg * 8:(reg + 1) * 8, :] = jnp.broadcast_to(row[:, _tile(c)], (8, LANES))
        buf[_AK + c, 0:HALO, :] = jnp.zeros((HALO, LANES), f32)
    w_copy(0).wait()
    for cp in (x_copy(1), ssmk_copy):
        cp.start()
    prepare_weight(0)

    q_scale = DH ** -0.5 * LOG2E
    x_copy(0).wait()
    projection(0, _Q, 0, NI // 2, gate_ops, gate, q_scale)
    for cp in (w_copy(1), ak_copy):
        cp.start()
    ssmk_copy.wait()
    for c in range(NT):
        for t in range(S // 256):
            buf[_FILT + c, HALO + t * 256:HALO + (t + 1) * 256, :] = (
                ssmk_v[_tile(c), t * 256:(t + 1) * 256].T.astype(f32))
    x_copy(1).wait()

    def q_work(i, zero):
        gate(i, zero)
        for h in range(2):
            first_stage(_FILT, 1, 2 * (i - NI // 2) + h, zero)

    projection(0, _Q, NI // 2, NI, gate_ops + 2 * stage_ops, q_work, q_scale)

    for cp in (av_copy, w_copy(2)):
        cp.start()
    w_copy(1).wait()
    prepare_weight(1)
    ak_copy.wait()

    def k_work(i, zero):
        widen_k(i * 2 * TM, zero)
        for h in range(2):
            first_stage(_FILT, 1, NI + 2 * i + h, zero)

    projection(1, _K, 0, NI // 2, 2 * TM // 32 * 30 + 2 * stage_ops, k_work)
    for cp in (gf_copy, gi_copy, wo_copy):
        cp.start()
    av_copy.wait()
    projection(1, _K, NI // 2, NI, 2 * TM // 16 * NT * 19,
               lambda i, zero: shift_conv((i - NI // 2) * 2 * TM, zero))
    fill_halo(_K)

    w_copy(2).wait()
    prepare_weight(2)

    def v_work(i, zero):
        for h in range(2):
            first_stage(_KV, 0, 2 * i + h, zero)
            for n in range(h * early // 2, (h + 1) * early // 2):
                scores(i, n)

    projection(2, _V, 0, NI, 2 * stage_ops + early * score_ops, v_work)
    fill_halo(_V)

    gf_copy.wait()
    gi_copy.wait()
    wo_copy.wait()
    for u in range(NT):
        reorder_rows(wo_v[:, _tile(u)], wop_v, u)

    def m_step(i, carry):
        zero = (i // NI) * 8
        same_head = (lane_head(0) == lane_head(1)).astype(bf16)

        def logit_rows(n, start, size):
            return _LOGITS + n // 4, rows_at(zero + (n % 4) * WIN * NB + start, size)

        def head_sums(n, v):
            logits = jnp.dot(part_v[i * steps + n, v * 2 * NB:(v + 1) * 2 * NB, :], same_head,
                             preferred_element_type=f32)

            def put(s):
                plane, rows = logit_rows(n, v * 2 * NB + s * 32, 32)
                buf[plane, rows, :] = logits[s * 32:(s + 1) * 32]
            return [(True, put)]

        def gate_sums(n):
            r0 = i * TM + n * 2 * NB
            z = jnp.dot(gate_v[pl.ds(pl.multiple_of(r0, 2 * NB), 2 * NB), :],
                        jnp.ones((LANES, LANES), bf16), preferred_element_type=f32)

            def put(s):
                buf[_GATE, rows_at(r0 + s * 32, 32), :] = 1.0 / (1.0 + jnp.exp(-z[s * 32:(s + 1) * 32]))
            return [(True, put)]

        def forward(n, c):
            j = i * steps + n
            f = jnp.dot(gf_v[j], res[j, :, 2 * c * LANES:2 * (c + 1) * LANES],
                        preferred_element_type=f32)
            groups = []
            for v in range(NB // 8):
                re, im = slice(v * 16, v * 16 + 8), slice(v * 16 + 8, v * 16 + 16)
                ur, ui, kr, ki = f[re, :LANES], f[im, :LANES], f[re, LANES:], f[im, LANES:]
                rr, ii = ur * kr, ui * ki
                pr, pi = rr - ii, ur * ki + ui * kr
                if n == steps - 1 and v == 0:
                    real = ((jax.lax.broadcasted_iota(jnp.int32, (8, LANES), 0) == 0)
                            & (i == NI - 1))
                    pr, pi = jnp.where(real, rr, pr), jnp.where(real, ii, pi)
                groups += [pr, pi]

            def mark(t, s):
                buf[_MISC, pl.ds(pl.multiple_of(zero + _DUMMY * 8, 8), 8), :] = (
                    f[s * 32 + 24:(s + 1) * 32, _tile(t)])
            return (jnp.concatenate(groups, axis=0).astype(bf16),
                    [(False, functools.partial(mark, t)) for t in range(2)])

        def inverse(n, c, prod):
            j = i * steps + n
            back = jnp.dot(gi_v[j], prod, preferred_element_type=f32)

            def put(s):
                buf[_SPEC + NT * (j // (NA // 2)) + c,
                    rows_at((j % (NA // 2)) * 2 * NB + s * 32, 32), :] = back[s * 32:(s + 1) * 32]
            return [(True, put)]

        def attend(n, v):
            r0 = i * TM + n * NB + v * 16
            halves = []
            for h in range(2):
                pacer.tick(26)
                lg = []
                for w in range(WIN):
                    plane, rows = logit_rows(n, (v * WIN + w) * 16 + h * 8, 8)
                    lg.append(buf[plane, rows, :])
                if n == 0 and v == 0:
                    pos = r0 + h * 8 + jax.lax.broadcasted_iota(jnp.int32, (8, LANES), 0)
                    lg = [jnp.where(pos >= DIL * w, l, -1e9 * LOG2E) for w, l in enumerate(lg)]
                top = functools.reduce(jnp.maximum, lg)
                p = [jnp.exp2(l - top) for l in lg]
                norm = (1.0 - buf[_GATE, rows_at(r0 + h * 8, 8), :]) / functools.reduce(jnp.add, p)
                outs = []
                for c in range(NT):
                    pacer.tick(17)
                    acc = None
                    for w in range(WIN):
                        term = p[w] * buf[_V + c, pl.ds(HALO + r0 + h * 8 - DIL * w, 8), :]
                        acc = term if acc is None else acc + term
                    outs.append(acc * norm)
                halves.append(outs)
            for c in range(NT):
                o_v[v, pl.ds(pl.multiple_of((i * steps + n) * 16, 16), 16), _tile(c)] = (
                    jnp.concatenate([halves[0][c], halves[1][c]], axis=0).astype(bf16))

        units, lag = steps * NT, 3
        jobs, ready, prods = sum((gate_sums(n) for n in range(4)), []), [], []
        for u in range(units + lag):
            while len(ready) < min(4 * steps, 4 + u * 4 // NT):
                jobs += head_sums(*divmod(len(ready), 4))
                ready.append(len(jobs))
            if u < units:
                prod, more = forward(*divmod(u, NT))
                prods.append(prod)
                jobs += more
            if u >= lag:
                jobs += inverse(*divmod(u - lag, NT), prods[u - lag])

        def store_round(group, s):
            for fn in [fn for keep, fn in group if keep] or [group[0][1]]:
                fn(s)

        stores = [functools.partial(store_round, jobs[r:r + 4], s)
                  for r in range(0, len(jobs), 4) for s in range(4)]
        pacer.start(stores, ((steps - early) * score_ops + steps * 8 * (26 + NT * 17)) * 1.04)
        for n in range(steps):
            for v in range(4):
                pacer.emit(-(-ready[4 * n + v] // 4) * 4)
                attend(n, v)
            if n % 2 == 1:
                scores(jnp.minimum(i + 1, NI - 1), early + n // 2)
        pacer.flush()
        return carry

    def first_scores(n, carry):
        scores(0, n)
        return carry

    jax.lax.fori_loop(early, steps, first_scores, 0)
    jax.lax.fori_loop(0, NI, m_step, 0)

    def w_step(i, carry):
        zero = (i // NI) * 8
        fft = _Fft(pacer, lambda k: misc(_COS + k, zero))
        mm = lambda rows, k, n: jnp.dot(o_v[i, rows, k], wop_v[k, n], preferred_element_type=f32)
        stores = matmul_stores(mm, _PROJ, zero)
        pacer.start(stores, NT * 2 * 484 + (NT - 1) * NA * 13)

        def mix(c):
            skip_c = misc(_SKIP + c, zero)
            skip_c = jnp.concatenate([skip_c, skip_c], axis=0)
            for a in range(NA):
                pacer.tick(13)
                row = pl.multiple_of(a * NB + i * 16, 16)
                y = y32[c, a * 16:(a + 1) * 16, :] + buf[_KV + c, rows_at(row, 16), :] * skip_c
                gated = buf[_GATE, rows_at(row, 16), :] * x_v[pl.ds(row, 16), _tile(c)].astype(f32)
                out_v[i, a, :, _tile(c)] = (
                    gated * y + buf[_PROJ + c, rows_at(zero + a * 16, 16), :]).astype(bf16)

        for c in range(NT):
            for h in range(2):
                def load(j):
                    pacer.tick()
                    plane = _SPEC + NT * (j // (NA // 2)) + c
                    row = (j % (NA // 2)) * 2 * NB + (2 * i + h) * 16
                    return ((buf[plane, rows_at(row, 8), :], 1), (buf[plane, rows_at(row + 8, 8), :], 1))

                blocks = [functools.partial(load, j) for j in range(NA)]
                even, odd = fft.even_bwd(blocks[NA // 2:]), fft.odd_bwd(blocks[:NA // 2])
                for a in range(NA):
                    y32[c, a * 16 + h * 8:a * 16 + (h + 1) * 8, :] = _value(fft.add(even[a], odd[a]))
            if c > 0:
                pacer.emit(len(stores) - (NT - c) * TM // 32)
                mix(c - 1)
        pacer.flush()
        mix(NT - 1)
        out_copy(i).start()
        return carry

    jax.lax.fori_loop(0, NI, w_step, 0)
    for i in range(NI):
        out_copy(i).wait()


@jax.jit
def pallas_gated_mix__ssm_conv_h3__sliding_local_dilated__prompt_kernel(
    A_q: jax.Array,
    A_k: jax.Array,
    A_v: jax.Array,
    A_shift_k: jax.Array,
    A_ssm_k: jax.Array,
    A_ssm_D: jax.Array,
    B_x: jax.Array,
    B_wqkv: jax.Array,
    B_wo: jax.Array,
    gate_w: jax.Array,
):
    del B_x
    assert A_q.shape == (1, S, D) and A_shift_k.shape == (D, KS)
    f32, bf16 = jnp.float32, jnp.bfloat16
    gf, gi = _dft_matrices()
    hbm = pl.BlockSpec(memory_space=pl.ANY)
    vmem = pl.BlockSpec(memory_space=pltpu.VMEM)
    out = pl.pallas_call(
        _kernel,
        out_shape=jax.ShapeDtypeStruct((NA, NB, D), bf16),
        in_specs=[hbm, hbm, hbm, vmem, hbm, vmem, hbm, hbm, vmem, hbm, hbm],
        out_specs=hbm,
        scratch_shapes=[
            pltpu.VMEM((S, D), bf16),
            pltpu.VMEM((S, D), bf16),
            pltpu.VMEM((S, D), bf16),
            pltpu.VMEM((D, S), bf16),
            pltpu.VMEM((3, D, D), bf16),
            pltpu.VMEM((3, D, D), bf16),
            pltpu.VMEM((D, D), bf16),
            pltpu.VMEM((D, D), bf16),
            pltpu.VMEM((NT, D // 2, LANES), jnp.uint32),
            pltpu.VMEM((NA, 2 * NB, 2 * NB), bf16),
            pltpu.VMEM((NA, 2 * NB, 2 * NB), bf16),
            pltpu.VMEM((_LOGITS + 2, HALO + S, LANES), f32),
            pltpu.VMEM((S, LANES), bf16),
            pltpu.VMEM((NA, 2 * NB, 2 * D), bf16),
            pltpu.VMEM((NA, WIN * NB, LANES), bf16),
            pltpu.VMEM((NT, TM, LANES), f32),
            pltpu.VMEM((NI, TM, D), bf16),
            pltpu.VMEM((NI, NA, 16, D), bf16),
            pltpu.SemaphoreType.DMA((9,)),
            pltpu.SemaphoreType.DMA((2,)),
            pltpu.SemaphoreType.DMA((NI,)),
        ],
        compiler_params=pltpu.CompilerParams(vmem_limit_bytes=110 * 1024 * 1024),
        name="gated_mix_h3_local_attn",
    )(A_q.reshape(S, D), A_k.reshape(S, D), A_v.reshape(S, D), A_shift_k.T, A_ssm_k,
      A_ssm_D, B_wqkv, B_wo, gate_w, gf, gi)
    return out.reshape(1, S, D)
```

```python
import functools
import math

import jax
import jax.numpy as jnp
import numpy as np
from jax.experimental import pallas as pl
from jax.experimental.pallas import tpu as pltpu

S = 2048
D = 640
H = 32
DH = D // H
WIN = 8
DIL = 2
KS = 4
LANES = 128
NT = D // LANES
NA = 32
NB = 64
HALO = 16
TM = 512
NI = S // TM


class _Pacer:
    def __init__(self):
        self.stores, self.done, self.ops, self.rate = [], 0, 0, 0.0

    def start(self, stores, vector_ops):
        self.flush()
        self.stores, self.done, self.ops = list(stores), 0, 0
        self.rate = len(self.stores) / vector_ops

    def tick(self, ops=0):
        self.emit(min(len(self.stores), int(self.ops * self.rate)))
        self.ops += ops

    def flush(self):
        self.emit(len(self.stores))

    def emit(self, due):
        while self.done < due:
            self.stores[self.done]()
            self.done += 1


def _neg(a):
    return (a[0], -a[1])


def _mul_i(x, s):
    return (_neg(x[1]), x[0]) if s > 0 else (x[1], _neg(x[0]))


class _Fft:
    def __init__(self, pacer, cosine):
        self.pacer = pacer
        self.cosine = cosine

    def add(self, a, b):
        self.pacer.ops += 1
        if a[1] == b[1]:
            return (a[0] + b[0], a[1])
        return (a[0] - b[0], 1) if a[1] > 0 else (b[0] - a[0], 1)

    def sub(self, a, b):
        return self.add(a, _neg(b))

    def mul(self, a, c):
        self.pacer.ops += 1
        return (a[0] * c[0], a[1] * c[1])

    def cadd(self, x, y):
        return (self.add(x[0], y[0]), self.add(x[1], y[1]))

    def csub(self, x, y):
        return (self.sub(x[0], y[0]), self.sub(x[1], y[1]))

    def cos(self, k):
        k = min(k % 64, -k % 64)
        return (self.cosine(k), 1) if k < 16 else (self.cosine(32 - k), -1)

    def twiddle(self, x, num, den):
        k = (num * (64 // den)) % 64
        if k % 16 == 0:
            for _ in range(k // 16):
                x = _mul_i(x, 1)
            return x
        self.pacer.tick()
        re, im = x
        c = self.cos(k)
        if k % 8 == 0:
            sc, ss = c[1], (1 if k < 32 else -1)
            pick = lambda v, sign: v if sign > 0 else _neg(v)
            return (self.mul(self.sub(pick(re, sc), pick(im, ss)), (c[0], 1)),
                    self.mul(self.add(pick(re, ss), pick(im, sc)), (c[0], 1)))
        s = self.cos(k - 16)
        return (self.sub(self.mul(re, c), self.mul(im, s)),
                self.add(self.mul(re, s), self.mul(im, c)))

    def cfft(self, z, sgn):
        n = len(z)
        if n == 1:
            return [z[0]()]
        if n == 2:
            a, b = z[0](), z[1]()
            return [self.cadd(a, b), self.csub(a, b)]
        ev, o1, o3 = self.cfft(z[0::2], sgn), self.cfft(z[1::4], sgn), self.cfft(z[3::4], sgn)
        out = [None] * n
        for r in range(n // 4):
            t1 = self.twiddle(o1[r], sgn * r, n)
            t3 = self.twiddle(o3[r], sgn * 3 * r, n)
            p, m = self.cadd(t1, t3), _mul_i(self.csub(t1, t3), sgn)
            lo, hi = ev[r], ev[r + n // 4]
            out[r], out[r + n // 2] = self.cadd(lo, p), self.csub(lo, p)
            out[r + n // 4], out[r + 3 * n // 4] = self.cadd(hi, m), self.csub(hi, m)
        return out

    def odd_fwd(self, d):
        m = len(d)
        return self.cfft([lambda a=a: self.twiddle((d[a](), _neg(d[a + m // 2]())), -a, 2 * m)
                          for a in range(m // 2)], -1)

    def odd_bwd(self, y):
        m = 2 * len(y)
        z = [self.twiddle(v, a, 2 * m) for a, v in enumerate(self.cfft(y, 1))]
        return [v[0] for v in z] + [_neg(v[1]) for v in z]

    def even_fwd(self, u):
        n = len(u)
        if n == 2:
            return [(u[0](), u[1]())]
        sums = [None] * (n // 2)

        def diff(a):
            lo, hi = u[a](), u[a + n // 2]()
            sums[a] = self.add(lo, hi)
            return self.sub(lo, hi)

        odd = self.odd_fwd([lambda a=a: diff(a) for a in range(n // 2)])
        return odd + self.even_fwd([lambda v=v: v for v in sums])

    def even_bwd(self, y):
        n = 2 * len(y)
        if n == 2:
            return list(y[0]())
        s, d = self.even_bwd(y[n // 4:]), self.odd_bwd(y[:n // 4])
        return [self.add(a, b) for a, b in zip(s, d)] + [self.sub(a, b) for a, b in zip(s, d)]


def _block_freqs():
    freqs = [4 * r + 1 for r in range(NA // 2)]
    n = NA
    while n > 2:
        freqs += [(4 * r + 1) * (2 * NA // n) for r in range(n // 4)]
        n //= 2
    return freqs + [None]


def _dft_matrices():
    fft = _Fft(_Pacer(), lambda k: 1.0)
    probe = [lambda: (1.0, 1)] * NA
    signs = [(re[1], im[1]) for re, im in fft.odd_fwd(probe) + fft.even_fwd(probe)]
    n = 2 * S
    b = np.arange(NB)
    k2 = np.arange(NB)[:, None]
    fwd = np.zeros((NA, 2 * NB, 2, NB))
    inv = np.zeros((NA, 2 * NB, 2, NB))
    for j, f in enumerate(_block_freqs()):
        weight = np.full((2 * NB, 1), 2.0 / n)
        if f is None:
            for part in range(2):
                ang = -2 * np.pi * ((k2 * (b + NB * part)) % (2 * NB)) / (2 * NB)
                fwd[j, :NB, part], fwd[j, NB:, part] = np.cos(ang), np.sin(ang)
                fwd[j, NB, part] = 1.0 - 2.0 * (b % 2)
            weight[0] = weight[NB] = 1.0 / n
        else:
            ang = -2 * np.pi * ((b * (f + 2 * NA * k2)) % n) / n
            fwd[j, :NB, 0], fwd[j, :NB, 1] = np.cos(ang), -np.sin(ang)
            fwd[j, NB:, 0], fwd[j, NB:, 1] = np.sin(ang), np.cos(ang)
        inv[j] = fwd[j] * weight[:, :, None]
        fwd[j] *= np.asarray(signs[j], np.float64)[None, :, None]
    order = lambda g: g.reshape(NA, 2, NB // 8, 8, 2, NB // 8, 8).transpose(
        0, 2, 1, 3, 5, 4, 6).reshape(NA, 2 * NB, 2 * NB)
    return (order(fwd).astype(jnp.bfloat16),
            order(inv).transpose(0, 2, 1).astype(jnp.bfloat16))


def _value(a):
    return a[0] if a[1] > 0 else -a[0]


_Q, _K, _V, _FILT, _AK, _KV, _MISC = (n * NT for n in range(7))
_GATE = _MISC + 1
_LOGITS = _MISC + 2
_SPEC = _FILT
_PROJ = _Q
_COS, _TAP, _SKIP, _GW, _DUMMY = 0, 16, 16 + KS * NT, 16 + (KS + 1) * NT, 16 + (KS + 2) * NT
LOG2E = math.log2(math.e)


def _tile(c):
    return slice(c * LANES, (c + 1) * LANES)


def _kernel(x_hbm, ak_hbm, av_hbm, shift_ref, ssmk_hbm, d_ref, wqkv_hbm, wo_hbm, gw_ref,
            gf_hbm, gi_hbm, out_hbm,
            x_v, ak_v, av_v, ssmk_v, w_v, wt_v, wo_v, wop_v, words, gf_v, gi_v,
            buf, gate_v, g_v, res, part_a, part_b, y32, o_v, out_v, sem_in, sem_x, sem_out):
    f32, bf16 = jnp.float32, jnp.bfloat16
    pacer = _Pacer()

    def w_copy(p):
        return pltpu.make_async_copy(wqkv_hbm.at[:, pl.ds(p * D, D)], w_v.at[p], sem_in.at[p])

    def x_copy(i):
        rows = pl.ds(pl.multiple_of(i * TM, TM), TM)
        return pltpu.make_async_copy(x_hbm.at[rows], x_v.at[rows], sem_x.at[i])

    ssmk_copy = pltpu.make_async_copy(ssmk_hbm, ssmk_v, sem_in.at[3])
    ak_copy = pltpu.make_async_copy(ak_hbm, ak_v, sem_in.at[4])
    av_copy = pltpu.make_async_copy(av_hbm, av_v, sem_in.at[5])
    gf_copy = pltpu.make_async_copy(gf_hbm, gf_v, sem_in.at[6])
    gi_copy = pltpu.make_async_copy(gi_hbm, gi_v, sem_in.at[7])
    wo_copy = pltpu.make_async_copy(wo_hbm, wo_v, sem_in.at[8])

    def out_copy(i):
        rows = pl.ds(pl.multiple_of(i * 16, 16), 16)
        return pltpu.make_async_copy(out_v.at[i], out_hbm.at[:, rows, :], sem_out.at[i])

    def rows_at(start, size):
        return pl.ds(pl.multiple_of(HALO + start, 8), size)

    def misc(reg, zero):
        return buf[_MISC, pl.ds(pl.multiple_of(zero + reg * 8, 8), 8), :]

    def reorder_rows(tile, dst, u):
        words[u] = pltpu.bitcast(tile, jnp.uint32)
        for pair in range(DH // 2):
            dst[pair * 2 * H:(pair + 1) * 2 * H, _tile(u)] = pltpu.bitcast(
                words[u, pl.ds(pair, H, stride=DH // 2), :], bf16)

    def prepare_weight(p):
        for u in range(NT):
            reorder_rows(w_v[p, _tile(u), :].T, wt_v.at[p], u)

    def matmul_stores(mm, plane, r0, scale=None):
        k_head, k_tail, quarter = slice(0, D - LANES), slice(D - LANES, D), TM // 4
        staged = mm(slice(0, TM), k_tail, k_head)
        last = [mm(slice(n * quarter, (n + 1) * quarter), k_tail, k_tail) for n in range(4)]
        full = [mm(slice(0, TM), k_head, _tile(c)) for c in range(NT)]

        def stage(v):
            for c in range(NT - 1):
                buf[plane + c, rows_at(r0 + v * 32, 32), :] = staged[v * 32:(v + 1) * 32, _tile(c)]

        def stage_last(v):
            for n in range(4):
                buf[plane + NT - 1, rows_at(r0 + n * quarter + v * 32, 32), :] = (
                    last[n][v * 32:(v + 1) * 32])

        def finish(c, v):
            rows = rows_at(r0 + v * 32, 32)
            val = full[c][v * 32:(v + 1) * 32] + buf[plane + c, rows, :]
            buf[plane + c, rows, :] = val if scale is None else val * scale

        return ([functools.partial(stage, v) for v in range(TM // 32)]
                + [functools.partial(stage_last, v) for v in range(quarter // 32)]
                + [functools.partial(finish, c, v) for c in range(NT) for v in range(TM // 32)])

    lane_head = lambda axis: (jax.lax.broadcasted_iota(jnp.int32, (LANES, LANES), axis) % (2 * H)) // 2

    def gate(i, zero):
        for v in range(TM // 16):
            pacer.tick(30)
            xs = x_v[pl.ds(pl.multiple_of(i * TM + v * 16, 16), 16), :].astype(f32)
            acc = None
            for c in range(NT):
                gw = misc(_GW + c, zero)
                term = xs[:, _tile(c)] * jnp.concatenate([gw, gw], axis=0)
                acc = term if acc is None else acc + term
            gate_v[pl.ds(pl.multiple_of(i * TM + v * 16, 16), 16), :] = acc.astype(bf16)

    def first_stage(plane, col, beta, zero):
        fft = _Fft(pacer, lambda k: misc(_COS + k, zero))
        r0 = pl.multiple_of(beta * 16, 16)
        for c in range(NT):
            def load(a):
                pacer.tick()
                return (buf[plane + c, rows_at(a * NB + beta * 8, 8), :], 1)

            for half, fn in enumerate((fft.odd_fwd, fft.even_fwd)):
                outs = fn([functools.partial(load, a) for a in range(NA)])
                for j, (re, im) in enumerate(outs):
                    res[half * (NA // 2) + j, pl.ds(r0, 16), _tile(2 * c + col)] = (
                        jnp.concatenate([re[0], im[0]], axis=0).astype(bf16))

    def widen_k(r0, zero):
        for v in range(2 * TM // 32):
            pacer.tick(30)
            wide = ak_v[pl.ds(pl.multiple_of(r0 + v * 32, 32), 32), :].astype(f32)
            for c in range(NT):
                buf[_AK + c, rows_at(r0 + v * 32, 32), :] = wide[:, _tile(c)]

    def shift_conv(r0, zero):
        for v in range(2 * TM // 16):
            row = pl.multiple_of(r0 + v * 16, 16)
            vals = av_v[pl.ds(row, 16), :].astype(f32)
            kv = []
            for c in range(NT):
                pacer.tick(19)
                acc = None
                for t in range(KS):
                    tap = misc(_TAP + t * NT + c, zero)
                    term = (buf[_AK + c, pl.ds(HALO + row - t, 16), :]
                            * jnp.concatenate([tap, tap], axis=0))
                    acc = term if acc is None else acc + term
                kv.append(acc * vals[:, _tile(c)])
            for c in range(NT):
                buf[_KV + c, rows_at(row, 16), :] = kv[c]

    def part(i, n):
        return (part_a if n < early else part_b).at[i * early + n % early]

    def scores(i, n):
        for v in range(4):
            r0 = i * TM + n * NB + v * 16
            q = [buf[_Q + c, rows_at(r0, 16), :] for c in range(NT)]
            for w in range(WIN):
                pacer.tick(19)
                acc = None
                for c in range(NT):
                    term = q[c] * buf[_K + c, pl.ds(HALO + r0 - DIL * w, 16), :]
                    acc = term if acc is None else acc + term
                part(i, n)[(v * WIN + w) * 16:(v * WIN + w + 1) * 16, :] = acc.astype(bf16)

    gate_ops, stage_ops, score_ops = TM // 16 * 30, NT * 452, 4 * WIN * 19
    steps = NA // NI
    early = steps // 2

    def projection(p, plane, lo, hi, vector_ops, work, scale=None):
        def step(i, carry):
            if p == 0:
                x_copy(i).wait()
            r0 = pl.multiple_of(i * TM, TM)

            def mm(rows, k, n):
                lhs = x_v[pl.ds(r0 + rows.start, rows.stop - rows.start), k]
                return jax.lax.dot_general(lhs, wt_v[p, n, k], (((1,), (1,)), ((), ())),
                                           preferred_element_type=f32)

            pacer.start(matmul_stores(mm, plane, r0, scale), vector_ops * 1.03)
            work(i, (i // NI) * 8)
            pacer.flush()
            return carry

        jax.lax.fori_loop(lo, hi, step, 0)

    def fill_halo(plane):
        for c in range(NT):
            buf[plane + c, 0:HALO, :] = jnp.broadcast_to(buf[plane + c, HALO:HALO + 1, :], (HALO, LANES))

    for cp in (w_copy(0), x_copy(0)):
        cp.start()
    for k in range(1, 16):
        buf[_MISC, (_COS + k) * 8:(_COS + k + 1) * 8, :] = jnp.full(
            (8, LANES), math.cos(2 * math.pi * k / 64), f32)
    rows = [shift_ref[...].astype(f32)[t:t + 1] for t in range(KS)]
    rows += [d_ref[...].astype(f32).reshape(1, D), gw_ref[...].astype(f32).reshape(1, D)]
    for c in range(NT):
        for n, row in enumerate(rows):
            reg = _TAP + n * NT + c
            buf[_MISC, reg * 8:(reg + 1) * 8, :] = jnp.broadcast_to(row[:, _tile(c)], (8, LANES))
        buf[_AK + c, 0:HALO, :] = jnp.zeros((HALO, LANES), f32)
    w_copy(0).wait()
    x_copy(1).start()
    prepare_weight(0)

    q_scale = DH ** -0.5 * LOG2E
    ssmk_copy.start()
    projection(0, _Q, 0, NI // 2, gate_ops, gate, q_scale)
    ssmk_copy.wait()
    for cp in (x_copy(2), x_copy(3), w_copy(1)):
        cp.start()
    for c in range(NT):
        for t in range(S // 256):
            buf[_FILT + c, HALO + t * 256:HALO + (t + 1) * 256, :] = (
                ssmk_v[_tile(c), t * 256:(t + 1) * 256].T.astype(f32))
    ak_copy.start()

    def q_work(i, zero):
        gate(i, zero)
        for h in range(2):
            first_stage(_FILT, 1, 2 * (i - NI // 2) + h, zero)

    projection(0, _Q, NI // 2, NI, gate_ops + 2 * stage_ops, q_work, q_scale)

    for cp in (av_copy, w_copy(2)):
        cp.start()
    w_copy(1).wait()
    prepare_weight(1)
    ak_copy.wait()

    def k_work(i, zero):
        widen_k(i * 2 * TM, zero)
        for h in range(2):
            first_stage(_FILT, 1, NI + 2 * i + h, zero)

    projection(1, _K, 0, NI // 2, 2 * TM // 32 * 30 + 2 * stage_ops, k_work)
    for cp in (gf_copy, gi_copy, wo_copy):
        cp.start()
    av_copy.wait()
    projection(1, _K, NI // 2, NI, 2 * TM // 16 * NT * 19,
               lambda i, zero: shift_conv((i - NI // 2) * 2 * TM, zero))
    fill_halo(_K)

    w_copy(2).wait()
    prepare_weight(2)

    def v_work(i, zero):
        for h in range(2):
            first_stage(_KV, 0, 2 * i + h, zero)
            for n in range(h * early // 2, (h + 1) * early // 2):
                scores(i, n)

    projection(2, _V, 0, NI, 2 * stage_ops + early * score_ops, v_work)
    fill_halo(_V)

    gf_copy.wait()
    gi_copy.wait()
    wo_copy.wait()
    for u in range(NT):
        reorder_rows(wo_v[:, _tile(u)], wop_v, u)

    def m_step(i, carry):
        zero = (i // NI) * 8
        same_head = (lane_head(0) == lane_head(1)).astype(bf16)

        def logit_rows(n, start, size):
            return _LOGITS + n // 4, rows_at(zero + (n % 4) * WIN * NB + start, size)

        def head_sums(n, v):
            logits = jnp.dot(part(i, n)[v * 2 * NB:(v + 1) * 2 * NB, :], same_head,
                             preferred_element_type=f32)

            def put(s):
                plane, rows = logit_rows(n, v * 2 * NB + s * 32, 32)
                buf[plane, rows, :] = logits[s * 32:(s + 1) * 32]
            return [(True, put)]

        def gate_sums(n):
            r0 = i * TM + n * 2 * NB
            z = jnp.dot(gate_v[pl.ds(pl.multiple_of(r0, 2 * NB), 2 * NB), :],
                        jnp.ones((LANES, LANES), bf16), preferred_element_type=f32)

            def put(s):
                buf[_GATE, rows_at(r0 + s * 32, 32), :] = z[s * 32:(s + 1) * 32]
            return [(True, put)]

        def forward(n, c):
            j = i * steps + n
            f = jnp.dot(gf_v[j], res[j, :, 2 * c * LANES:2 * (c + 1) * LANES],
                        preferred_element_type=f32)
            groups = []
            for v in range(NB // 8):
                re, im = slice(v * 16, v * 16 + 8), slice(v * 16 + 8, v * 16 + 16)
                ur, ui, kr, ki = f[re, :LANES], f[im, :LANES], f[re, LANES:], f[im, LANES:]
                rr, ii = ur * kr, ui * ki
                pr, pi = rr - ii, ur * ki + ui * kr
                if n == steps - 1 and v == 0:
                    real = ((jax.lax.broadcasted_iota(jnp.int32, (8, LANES), 0) == 0)
                            & (i == NI - 1))
                    pr, pi = jnp.where(real, rr, pr), jnp.where(real, ii, pi)
                groups += [pr, pi]

            def mark(t, s):
                buf[_MISC, pl.ds(pl.multiple_of(zero + _DUMMY * 8, 8), 8), :] = (
                    f[s * 32 + 24:(s + 1) * 32, _tile(t)])
            return (jnp.concatenate(groups, axis=0).astype(bf16),
                    [(False, functools.partial(mark, t)) for t in range(2)])

        def inverse(n, c, prod):
            j = i * steps + n
            back = jnp.dot(gi_v[j], prod, preferred_element_type=f32)

            def put(s):
                buf[_SPEC + NT * (j // (NA // 2)) + c,
                    rows_at((j % (NA // 2)) * 2 * NB + s * 32, 32), :] = back[s * 32:(s + 1) * 32]
            return [(True, put)]

        def attend(n, v):
            r0 = i * TM + n * NB + v * 16
            halves = []
            for h in range(2):
                pacer.tick(36)
                lg = []
                for w in range(WIN):
                    plane, rows = logit_rows(n, (v * WIN + w) * 16 + h * 8, 8)
                    lg.append(buf[plane, rows, :])
                if n == 0 and v == 0:
                    pos = r0 + h * 8 + jax.lax.broadcasted_iota(jnp.int32, (8, LANES), 0)
                    lg = [jnp.where(pos >= DIL * w, l, -1e9 * LOG2E) for w, l in enumerate(lg)]
                top = functools.reduce(jnp.maximum, lg)
                p = [jnp.exp2(l - top) for l in lg]
                g = 1.0 / (1.0 + jnp.exp(-buf[_GATE, rows_at(r0 + h * 8, 8), :]))
                g_v[pl.ds(pl.multiple_of(r0 + h * 8, 8), 8), :] = g
                norm = (1.0 - g) / functools.reduce(jnp.add, p)
                outs = []
                for c in range(NT):
                    pacer.tick(17)
                    acc = None
                    for w in range(WIN):
                        term = p[w] * buf[_V + c, pl.ds(HALO + r0 + h * 8 - DIL * w, 8), :]
                        acc = term if acc is None else acc + term
                    outs.append(acc * norm)
                halves.append(outs)
            for c in range(NT):
                o_v[v, pl.ds(pl.multiple_of((i * steps + n) * 16, 16), 16), _tile(c)] = (
                    jnp.concatenate([halves[0][c], halves[1][c]], axis=0).astype(bf16))

        units, lag = steps * NT, 3
        jobs, ready, prods = sum((gate_sums(n) for n in range(4)), []), [], []
        for u in range(units + lag):
            while len(ready) < min(4 * steps, 4 + 2 * u, 12 + u * 4 // NT):
                jobs += head_sums((len(ready) // 4 + early) % steps, len(ready) % 4)
                ready.append(len(jobs))
            if u < units:
                prod, more = forward(*divmod(u, NT))
                prods.append(prod)
                jobs += more
            if u >= lag:
                jobs += inverse(*divmod(u - lag, NT), prods[u - lag])

        def store_round(group, s):
            for fn in [fn for keep, fn in group if keep] or [group[0][1]]:
                fn(s)

        stores = [functools.partial(store_round, jobs[r:r + 4], s)
                  for r in range(0, len(jobs), 4) for s in range(4)]
        pacer.start(stores, ((steps - early) * score_ops + steps * 8 * (36 + NT * 17)) * 1.04)
        later = [2, 3, 5, 7]
        for m in range(steps):
            for v in range(4):
                pacer.emit(-(-ready[4 * m + v] // 4) * 4)
                attend((m + early) % steps, v)
            if m in later:
                scores(jnp.minimum(i + 1, NI - 1), early + later.index(m))
        pacer.flush()
        return carry

    for n in range(early, steps):
        scores(0, n)
    jax.lax.fori_loop(0, NI, m_step, 0)

    def w_step(i, carry):
        zero = (i // NI) * 8
        fft = _Fft(pacer, lambda k: misc(_COS + k, zero))
        mm = lambda rows, k, n: jnp.dot(o_v[i, rows, k], wop_v[k, n], preferred_element_type=f32)
        stores = matmul_stores(mm, _PROJ, zero)
        pacer.start(stores, NT * (2 * 452 + NA * 15) * 1.15)

        signs = [None, None]

        def mix(c):
            skip_c = misc(_SKIP + c, zero)
            skip_c = jnp.concatenate([skip_c, skip_c], axis=0)
            for a in range(NA):
                pacer.tick(13)
                pacer.emit(len(stores) - (NT - c) * TM // 32 + a // 2 + 1)
                row = pl.multiple_of(a * NB + i * 16, 16)
                staged = pl.ds(pl.multiple_of(2 * zero + a * 16, 8), 16)
                y = (buf[_KV + c, rows_at(row, 16), :] * skip_c, 1)
                for half in range(2):
                    y = fft.add(y, (y32[half, c, staged, :], signs[half][a]))
                y = _value(y)
                branch = y * x_v[pl.ds(row, 16), _tile(c)].astype(f32)
                out_v[i, a, :, _tile(c)] = (
                    branch * g_v[pl.ds(row, 16), :]
                    + buf[_PROJ + c, rows_at(zero + a * 16, 16), :]).astype(bf16)

        for c in range(NT):
            for h in range(2):
                def load(j):
                    pacer.tick()
                    plane = _SPEC + NT * (j // (NA // 2)) + c
                    row = (j % (NA // 2)) * 2 * NB + (2 * i + h) * 16
                    return ((buf[plane, rows_at(row, 8), :], 1), (buf[plane, rows_at(row + 8, 8), :], 1))

                blocks = [functools.partial(load, j) for j in range(NA)]
                for half, fn in enumerate((fft.odd_bwd, fft.even_bwd)):
                    outs = fn(blocks[half * NA // 2:(half + 1) * NA // 2])
                    signs[half] = [sign for _, sign in outs]
                    for a, (val, _) in enumerate(outs):
                        y32[half, c, pl.ds(pl.multiple_of(zero + a * 16 + h * 8, 8), 8), :] = val
            if c >= 2:
                mix(c - 2)
        mix(NT - 2)
        mix(NT - 1)
        pacer.flush()
        out_copy(i).start()
        return carry

    jax.lax.fori_loop(0, NI, w_step, 0)
    for i in range(NI):
        out_copy(i).wait()


@jax.jit
def pallas_gated_mix__ssm_conv_h3__sliding_local_dilated__prompt_kernel(
    A_q: jax.Array,
    A_k: jax.Array,
    A_v: jax.Array,
    A_shift_k: jax.Array,
    A_ssm_k: jax.Array,
    A_ssm_D: jax.Array,
    B_x: jax.Array,
    B_wqkv: jax.Array,
    B_wo: jax.Array,
    gate_w: jax.Array,
):
    del B_x
    assert A_q.shape == (1, S, D) and A_shift_k.shape == (D, KS)
    f32, bf16 = jnp.float32, jnp.bfloat16
    gf, gi = _dft_matrices()
    hbm = pl.BlockSpec(memory_space=pl.ANY)
    vmem = pl.BlockSpec(memory_space=pltpu.VMEM)
    out = pl.pallas_call(
        _kernel,
        out_shape=jax.ShapeDtypeStruct((NA, NB, D), bf16),
        in_specs=[hbm, hbm, hbm, vmem, hbm, vmem, hbm, hbm, vmem, hbm, hbm],
        out_specs=hbm,
        scratch_shapes=[
            pltpu.VMEM((S, D), bf16),
            pltpu.VMEM((S, D), bf16),
            pltpu.VMEM((S, D), bf16),
            pltpu.VMEM((D, S), bf16),
            pltpu.VMEM((3, D, D), bf16),
            pltpu.VMEM((3, D, D), bf16),
            pltpu.VMEM((D, D), bf16),
            pltpu.VMEM((D, D), bf16),
            pltpu.VMEM((NT, D // 2, LANES), jnp.uint32),
            pltpu.VMEM((NA, 2 * NB, 2 * NB), bf16),
            pltpu.VMEM((NA, 2 * NB, 2 * NB), bf16),
            pltpu.VMEM((_LOGITS + 2, HALO + S, LANES), f32),
            pltpu.VMEM((S, LANES), bf16),
            pltpu.VMEM((S, LANES), f32),
            pltpu.VMEM((NA, 2 * NB, 2 * D), bf16),
            pltpu.VMEM((NA // 2, WIN * NB, LANES), bf16),
            pltpu.VMEM((NA // 2, WIN * NB, LANES), bf16),
            pltpu.VMEM((2, NT, TM, LANES), f32),
            pltpu.VMEM((NI, TM, D), bf16),
            pltpu.VMEM((NI, NA, 16, D), bf16),
            pltpu.SemaphoreType.DMA((9,)),
            pltpu.SemaphoreType.DMA((NI,)),
            pltpu.SemaphoreType.DMA((NI,)),
        ],
        compiler_params=pltpu.CompilerParams(vmem_limit_bytes=110 * 1024 * 1024),
        name="gated_mix_h3_local_attn",
    )(A_q.reshape(S, D), A_k.reshape(S, D), A_v.reshape(S, D), A_shift_k.T, A_ssm_k,
      A_ssm_D, B_wqkv, B_wo, gate_w, gf, gi)
    return out.reshape(1, S, D)
```

```python
import functools
import math

import jax
import jax.numpy as jnp
import numpy as np
from jax.experimental import pallas as pl
from jax.experimental.pallas import tpu as pltpu

S = 2048
D = 640
H = 32
DH = D // H
WIN = 8
DIL = 2
KS = 4
LANES = 128
NT = D // LANES
NA = 32
NB = 64
HALO = 16
TM = 512
NI = S // TM


class _Pacer:
    def __init__(self):
        self.stores, self.done, self.ops, self.rate = [], 0, 0, 0.0

    def start(self, stores, vector_ops):
        self.flush()
        self.stores, self.done, self.ops = list(stores), 0, 0
        self.rate = len(self.stores) / vector_ops

    def tick(self, ops=0):
        self.emit(min(len(self.stores), int(self.ops * self.rate)))
        self.ops += ops

    def flush(self):
        self.emit(len(self.stores))

    def emit(self, due):
        while self.done < due:
            self.stores[self.done]()
            self.done += 1


def _neg(a):
    return (a[0], -a[1])


def _mul_i(x, s):
    return (_neg(x[1]), x[0]) if s > 0 else (x[1], _neg(x[0]))


class _Fft:
    def __init__(self, pacer, cosine):
        self.pacer = pacer
        self.cosine = cosine

    def add(self, a, b):
        self.pacer.ops += 1
        if a[1] == b[1]:
            return (a[0] + b[0], a[1])
        return (a[0] - b[0], 1) if a[1] > 0 else (b[0] - a[0], 1)

    def sub(self, a, b):
        return self.add(a, _neg(b))

    def mul(self, a, c):
        self.pacer.ops += 1
        return (a[0] * c[0], a[1] * c[1])

    def cadd(self, x, y):
        return (self.add(x[0], y[0]), self.add(x[1], y[1]))

    def csub(self, x, y):
        return (self.sub(x[0], y[0]), self.sub(x[1], y[1]))

    def cos(self, k):
        k = min(k % 64, -k % 64)
        return (self.cosine(k), 1) if k < 16 else (self.cosine(32 - k), -1)

    def twiddle(self, x, num, den):
        k = (num * (64 // den)) % 64
        if k % 16 == 0:
            for _ in range(k // 16):
                x = _mul_i(x, 1)
            return x
        self.pacer.tick()
        re, im = x
        c = self.cos(k)
        if k % 8 == 0:
            sc, ss = c[1], (1 if k < 32 else -1)
            pick = lambda v, sign: v if sign > 0 else _neg(v)
            return (self.mul(self.sub(pick(re, sc), pick(im, ss)), (c[0], 1)),
                    self.mul(self.add(pick(re, ss), pick(im, sc)), (c[0], 1)))
        s = self.cos(k - 16)
        return (self.sub(self.mul(re, c), self.mul(im, s)),
                self.add(self.mul(re, s), self.mul(im, c)))

    def cfft(self, z, sgn):
        n = len(z)
        if n == 1:
            return [z[0]()]
        if n == 2:
            a, b = z[0](), z[1]()
            return [self.cadd(a, b), self.csub(a, b)]
        ev, o1, o3 = self.cfft(z[0::2], sgn), self.cfft(z[1::4], sgn), self.cfft(z[3::4], sgn)
        out = [None] * n
        for r in range(n // 4):
            t1 = self.twiddle(o1[r], sgn * r, n)
            t3 = self.twiddle(o3[r], sgn * 3 * r, n)
            p, m = self.cadd(t1, t3), _mul_i(self.csub(t1, t3), sgn)
            lo, hi = ev[r], ev[r + n // 4]
            out[r], out[r + n // 2] = self.cadd(lo, p), self.csub(lo, p)
            out[r + n // 4], out[r + 3 * n // 4] = self.cadd(hi, m), self.csub(hi, m)
        return out

    def odd_fwd(self, d):
        m = len(d)
        return self.cfft([lambda a=a: self.twiddle((d[a](), _neg(d[a + m // 2]())), -a, 2 * m)
                          for a in range(m // 2)], -1)

    def odd_bwd(self, y):
        m = 2 * len(y)
        z = [self.twiddle(v, a, 2 * m) for a, v in enumerate(self.cfft(y, 1))]
        return [v[0] for v in z] + [_neg(v[1]) for v in z]

    def even_fwd(self, u):
        n = len(u)
        if n == 2:
            return [(u[0](), u[1]())]
        sums = [None] * (n // 2)

        def diff(a):
            lo, hi = u[a](), u[a + n // 2]()
            sums[a] = self.add(lo, hi)
            return self.sub(lo, hi)

        odd = self.odd_fwd([lambda a=a: diff(a) for a in range(n // 2)])
        return odd + self.even_fwd([lambda v=v: v for v in sums])

    def even_bwd(self, y):
        n = 2 * len(y)
        if n == 2:
            return list(y[0]())
        s, d = self.even_bwd(y[n // 4:]), self.odd_bwd(y[:n // 4])
        return [self.add(a, b) for a, b in zip(s, d)] + [self.sub(a, b) for a, b in zip(s, d)]


def _block_freqs():
    freqs = [4 * r + 1 for r in range(NA // 2)]
    n = NA
    while n > 2:
        freqs += [(4 * r + 1) * (2 * NA // n) for r in range(n // 4)]
        n //= 2
    return freqs + [None]


def _dft_matrices():
    fft = _Fft(_Pacer(), lambda k: 1.0)
    probe = [lambda: (1.0, 1)] * NA
    signs = [(re[1], im[1]) for re, im in fft.odd_fwd(probe) + fft.even_fwd(probe)]
    n = 2 * S
    b = np.arange(NB)
    k2 = np.arange(NB)[:, None]
    fwd = np.zeros((NA, 2 * NB, 2, NB))
    inv = np.zeros((NA, 2 * NB, 2, NB))
    for j, f in enumerate(_block_freqs()):
        weight = np.full((2 * NB, 1), 2.0 / n)
        if f is None:
            for part in range(2):
                ang = -2 * np.pi * ((k2 * (b + NB * part)) % (2 * NB)) / (2 * NB)
                fwd[j, :NB, part], fwd[j, NB:, part] = np.cos(ang), np.sin(ang)
                fwd[j, NB, part] = 1.0 - 2.0 * (b % 2)
            weight[0] = weight[NB] = 1.0 / n
        else:
            ang = -2 * np.pi * ((b * (f + 2 * NA * k2)) % n) / n
            fwd[j, :NB, 0], fwd[j, :NB, 1] = np.cos(ang), -np.sin(ang)
            fwd[j, NB:, 0], fwd[j, NB:, 1] = np.sin(ang), np.cos(ang)
        inv[j] = fwd[j] * weight[:, :, None]
        fwd[j] *= np.asarray(signs[j], np.float64)[None, :, None]
    order = lambda g: g.reshape(NA, 2, NB // 8, 8, 2, NB // 8, 8).transpose(
        0, 2, 1, 3, 5, 4, 6).reshape(NA, 2 * NB, 2 * NB)
    return (order(fwd).astype(jnp.bfloat16),
            order(inv).transpose(0, 2, 1).astype(jnp.bfloat16))


def _value(a):
    return a[0] if a[1] > 0 else -a[0]


_Q, _K, _V, _FILT, _AK, _KV, _MISC = (n * NT for n in range(7))
_GATE = _MISC + 1
_LOGITS = _MISC + 2
_SPEC = _FILT
_PROJ = _Q
_COS, _TAP, _SKIP, _GW, _DUMMY = 0, 16, 16 + KS * NT, 16 + (KS + 1) * NT, 16 + (KS + 2) * NT
LOG2E = math.log2(math.e)


def _tile(c):
    return slice(c * LANES, (c + 1) * LANES)


def _kernel(x_hbm, ak_hbm, av_hbm, shift_ref, ssmk_hbm, d_ref, wqkv_hbm, wo_hbm, gw_ref,
            gf_hbm, gi_hbm, out_hbm,
            x_v, ak_v, av_v, ssmk_v, w_v, wt_v, wo_v, wop_v, words, gf_v, gi_v,
            buf, gate_v, g_v, res, part_a, part_b, y32, o_v, out_v, sem_in, sem_x, sem_out):
    f32, bf16 = jnp.float32, jnp.bfloat16
    pacer = _Pacer()

    def w_copy(p):
        return pltpu.make_async_copy(wqkv_hbm.at[:, pl.ds(p * D, D)], w_v.at[p], sem_in.at[p])

    def x_copy(i):
        rows = pl.ds(pl.multiple_of(i * TM, TM), TM)
        return pltpu.make_async_copy(x_hbm.at[rows], x_v.at[rows], sem_x.at[i])

    ssmk_copy = pltpu.make_async_copy(ssmk_hbm, ssmk_v, sem_in.at[3])
    ak_copy = pltpu.make_async_copy(ak_hbm, ak_v, sem_in.at[4])
    av_copy = pltpu.make_async_copy(av_hbm, av_v, sem_in.at[5])
    gf_copy = pltpu.make_async_copy(gf_hbm, gf_v, sem_in.at[6])
    gi_copy = pltpu.make_async_copy(gi_hbm, gi_v, sem_in.at[7])
    wo_copy = pltpu.make_async_copy(wo_hbm, wo_v, sem_in.at[8])

    def out_copy(i):
        rows = pl.ds(pl.multiple_of(i * 16, 16), 16)
        return pltpu.make_async_copy(out_v.at[i], out_hbm.at[:, rows, :], sem_out.at[i])

    def rows_at(start, size):
        return pl.ds(pl.multiple_of(HALO + start, 8), size)

    def misc(reg, zero):
        return buf[_MISC, pl.ds(pl.multiple_of(zero + reg * 8, 8), 8), :]

    def reorder_rows(tile, dst, u):
        words[u] = pltpu.bitcast(tile, jnp.uint32)
        for pair in range(DH // 2):
            dst[pair * 2 * H:(pair + 1) * 2 * H, _tile(u)] = pltpu.bitcast(
                words[u, pl.ds(pair, H, stride=DH // 2), :], bf16)

    def prepare_weight(p):
        for u in range(NT):
            reorder_rows(w_v[p, _tile(u), :].T, wt_v.at[p], u)

    def matmul_stores(mm, plane, r0, scale=None):
        k_head, k_tail, quarter = slice(0, D - LANES), slice(D - LANES, D), TM // 4
        staged = mm(slice(0, TM), k_tail, k_head)
        last = [mm(slice(n * quarter, (n + 1) * quarter), k_tail, k_tail) for n in range(4)]
        full = [mm(slice(0, TM), k_head, _tile(c)) for c in range(NT)]

        def stage(v):
            for c in range(NT - 1):
                buf[plane + c, rows_at(r0 + v * 32, 32), :] = staged[v * 32:(v + 1) * 32, _tile(c)]

        def stage_last(v):
            for n in range(4):
                buf[plane + NT - 1, rows_at(r0 + n * quarter + v * 32, 32), :] = (
                    last[n][v * 32:(v + 1) * 32])

        def finish(c, v):
            rows = rows_at(r0 + v * 32, 32)
            val = full[c][v * 32:(v + 1) * 32] + buf[plane + c, rows, :]
            buf[plane + c, rows, :] = val if scale is None else val * scale

        return ([functools.partial(stage, v) for v in range(TM // 32)]
                + [functools.partial(stage_last, v) for v in range(quarter // 32)]
                + [functools.partial(finish, c, v) for c in range(NT) for v in range(TM // 32)])

    lane_head = lambda axis: (jax.lax.broadcasted_iota(jnp.int32, (LANES, LANES), axis) % (2 * H)) // 2

    def gate(i, zero, v):
        pacer.tick(30)
        rows = pl.ds(pl.multiple_of(i * TM + v * 16, 16), 16)
        xs = x_v[rows, :].astype(f32)
        acc = None
        for c in range(NT):
            gw = misc(_GW + c, zero)
            term = xs[:, _tile(c)] * jnp.concatenate([gw, gw], axis=0)
            acc = term if acc is None else acc + term
        gate_v[rows, :] = acc.astype(bf16)

    def first_stage(plane, col, pair, zero, side, chunks=1):
        fft = _Fft(pacer, lambda k: misc(_COS + k, zero))
        for slot in range(2 * NT):
            if slot % (2 * NT // chunks) == 0:
                n = slot // (2 * NT // chunks)
                for job in side[n * len(side) // chunks:(n + 1) * len(side) // chunks]:
                    job()
            beta, c = 2 * pair + slot // NT, slot % NT
            r0 = pl.multiple_of(beta * 16, 16)

            def load(a):
                pacer.tick()
                return (buf[plane + c, rows_at(a * NB + beta * 8, 8), :], 1)

            for half, fn in enumerate((fft.odd_fwd, fft.even_fwd)):
                outs = fn([functools.partial(load, a) for a in range(NA)])
                for j, (re, im) in enumerate(outs):
                    res[half * (NA // 2) + j, pl.ds(r0, 16), _tile(2 * c + col)] = (
                        jnp.concatenate([re[0], im[0]], axis=0).astype(bf16))

    def widen_k(r0):
        pacer.tick(30)
        wide = ak_v[pl.ds(pl.multiple_of(r0, 32), 32), :].astype(f32)
        for c in range(NT):
            buf[_AK + c, rows_at(r0, 32), :] = wide[:, _tile(c)]

    def shift_conv(r0, zero):
        for v in range(2 * TM // 16):
            row = pl.multiple_of(r0 + v * 16, 16)
            vals = av_v[pl.ds(row, 16), :].astype(f32)
            kv = []
            for c in range(NT):
                pacer.tick(19)
                acc = None
                for t in range(KS):
                    tap = misc(_TAP + t * NT + c, zero)
                    term = (buf[_AK + c, pl.ds(HALO + row - t, 16), :]
                            * jnp.concatenate([tap, tap], axis=0))
                    acc = term if acc is None else acc + term
                kv.append(acc * vals[:, _tile(c)])
            for c in range(NT):
                buf[_KV + c, rows_at(row, 16), :] = kv[c]

    def part(i, n):
        return (part_a if n < early else part_b).at[i * early + n % early]

    def scores(i, n, groups=range(4)):
        for v in groups:
            r0 = i * TM + n * NB + v * 16
            q = [buf[_Q + c, rows_at(r0, 16), :] for c in range(NT)]
            for w in range(WIN):
                pacer.tick(19)
                acc = None
                for c in range(NT):
                    term = q[c] * buf[_K + c, pl.ds(HALO + r0 - DIL * w, 16), :]
                    acc = term if acc is None else acc + term
                part(i, n)[(v * WIN + w) * 16:(v * WIN + w + 1) * 16, :] = acc.astype(bf16)

    gate_ops, stage_ops, score_ops = TM // 16 * 30, NT * 452, 4 * WIN * 19
    steps = NA // NI
    early = steps // 2

    def projection(p, plane, lo, hi, vector_ops, work, scale=None):
        def step(i, carry):
            if p == 0:
                x_copy(i).wait()
            r0 = pl.multiple_of(i * TM, TM)

            def mm(rows, k, n):
                lhs = x_v[pl.ds(r0 + rows.start, rows.stop - rows.start), k]
                return jax.lax.dot_general(lhs, wt_v[p, n, k], (((1,), (1,)), ((), ())),
                                           preferred_element_type=f32)

            pacer.start(matmul_stores(mm, plane, r0, scale), vector_ops * 1.02)
            work(i, (i // NI) * 8)
            pacer.flush()
            return carry

        jax.lax.fori_loop(lo, hi, step, 0)

    def fill_halo(plane):
        for c in range(NT):
            buf[plane + c, 0:HALO, :] = jnp.broadcast_to(buf[plane + c, HALO:HALO + 1, :], (HALO, LANES))

    for cp in (w_copy(0), x_copy(0)):
        cp.start()
    for k in range(1, 16):
        buf[_MISC, (_COS + k) * 8:(_COS + k + 1) * 8, :] = jnp.full(
            (8, LANES), math.cos(2 * math.pi * k / 64), f32)
    rows = [shift_ref[...].astype(f32)[t:t + 1] for t in range(KS)]
    rows += [d_ref[...].astype(f32).reshape(1, D), gw_ref[...].astype(f32).reshape(1, D)]
    for c in range(NT):
        for n, row in enumerate(rows):
            reg = _TAP + n * NT + c
            buf[_MISC, reg * 8:(reg + 1) * 8, :] = jnp.broadcast_to(row[:, _tile(c)], (8, LANES))
        buf[_AK + c, 0:HALO, :] = jnp.zeros((HALO, LANES), f32)
    w_copy(0).wait()
    x_copy(1).start()
    prepare_weight(0)

    q_scale = DH ** -0.5 * LOG2E
    ssmk_copy.start()
    gates = lambda i, zero: [functools.partial(gate, i, zero, v) for v in range(TM // 16)]
    projection(0, _Q, 0, NI // 2, gate_ops, lambda i, zero: [job() for job in gates(i, zero)], q_scale)
    ssmk_copy.wait()
    for cp in (x_copy(2), x_copy(3), w_copy(1)):
        cp.start()
    for c in range(NT):
        for t in range(S // 256):
            buf[_FILT + c, HALO + t * 256:HALO + (t + 1) * 256, :] = (
                ssmk_v[_tile(c), t * 256:(t + 1) * 256].T.astype(f32))
    ak_copy.start()

    def q_work(i, zero):
        first_stage(_FILT, 1, i - NI // 2, zero, gates(i, zero))

    projection(0, _Q, NI // 2, NI, gate_ops + 2 * stage_ops, q_work, q_scale)

    for cp in (av_copy, w_copy(2)):
        cp.start()
    w_copy(1).wait()
    prepare_weight(1)
    ak_copy.wait()

    def k_work(i, zero):
        first_stage(_FILT, 1, NI // 2 + i, zero,
                    [functools.partial(widen_k, i * 2 * TM + v * 32) for v in range(2 * TM // 32)])

    projection(1, _K, 0, NI // 2, 2 * TM // 32 * 30 + 2 * stage_ops, k_work)
    for cp in (gf_copy, gi_copy, wo_copy):
        cp.start()
    av_copy.wait()
    projection(1, _K, NI // 2, NI, 2 * TM // 16 * NT * 19,
               lambda i, zero: shift_conv((i - NI // 2) * 2 * TM, zero))
    fill_halo(_K)

    w_copy(2).wait()
    prepare_weight(2)

    def v_work(i, zero):
        first_stage(_KV, 0, i, zero,
                    [functools.partial(scores, i, n, [v]) for n in range(early) for v in range(4)], 2)

    projection(2, _V, 0, NI, 2 * stage_ops + early * score_ops, v_work)
    fill_halo(_V)

    gf_copy.wait()
    gi_copy.wait()
    wo_copy.wait()
    for u in range(NT):
        reorder_rows(wo_v[:, _tile(u)], wop_v, u)

    def m_step(i, carry):
        zero = (i // NI) * 8
        same_head = (lane_head(0) == lane_head(1)).astype(bf16)

        def logit_rows(n, start, size):
            return _LOGITS + n // 4, rows_at(zero + (n % 4) * WIN * NB + start, size)

        def head_sums(n, v):
            logits = jnp.dot(part(i, n)[v * 2 * NB:(v + 1) * 2 * NB, :], same_head,
                             preferred_element_type=f32)

            def put(s):
                plane, rows = logit_rows(n, v * 2 * NB + s * 32, 32)
                buf[plane, rows, :] = logits[s * 32:(s + 1) * 32]
            return [(True, put)]

        def gate_sums(n):
            r0 = i * TM + n * 2 * NB
            z = jnp.dot(gate_v[pl.ds(pl.multiple_of(r0, 2 * NB), 2 * NB), :],
                        jnp.ones((LANES, LANES), bf16), preferred_element_type=f32)

            def put(s):
                buf[_GATE, rows_at(r0 + s * 32, 32), :] = z[s * 32:(s + 1) * 32]
            return [(True, put)]

        def forward(n, c):
            j = i * steps + n
            f = jnp.dot(gf_v[j], res[j, :, 2 * c * LANES:2 * (c + 1) * LANES],
                        preferred_element_type=f32)
            groups = []
            for v in range(NB // 8):
                re, im = slice(v * 16, v * 16 + 8), slice(v * 16 + 8, v * 16 + 16)
                ur, ui, kr, ki = f[re, :LANES], f[im, :LANES], f[re, LANES:], f[im, LANES:]
                rr, ii = ur * kr, ui * ki
                pr, pi = rr - ii, ur * ki + ui * kr
                if n == steps - 1 and v == 0:
                    real = ((jax.lax.broadcasted_iota(jnp.int32, (8, LANES), 0) == 0)
                            & (i == NI - 1))
                    pr, pi = jnp.where(real, rr, pr), jnp.where(real, ii, pi)
                groups += [pr, pi]

            def mark(t, s):
                buf[_MISC, pl.ds(pl.multiple_of(zero + _DUMMY * 8, 8), 8), :] = (
                    f[s * 32 + 24:(s + 1) * 32, _tile(t)])
            return (jnp.concatenate(groups, axis=0).astype(bf16),
                    [(False, functools.partial(mark, t)) for t in range(2)])

        def inverse(n, c, prod):
            j = i * steps + n
            back = jnp.dot(gi_v[j], prod, preferred_element_type=f32)

            def put(s):
                buf[_SPEC + NT * (j // (NA // 2)) + c,
                    rows_at((j % (NA // 2)) * 2 * NB + s * 32, 32), :] = back[s * 32:(s + 1) * 32]
            return [(True, put)]

        def attend(n, v):
            r0 = i * TM + n * NB + v * 16
            halves = []
            for h in range(2):
                pacer.tick(36)
                lg = []
                for w in range(WIN):
                    plane, rows = logit_rows(n, (v * WIN + w) * 16 + h * 8, 8)
                    lg.append(buf[plane, rows, :])
                if n == 0 and v == 0:
                    pos = r0 + h * 8 + jax.lax.broadcasted_iota(jnp.int32, (8, LANES), 0)
                    lg = [jnp.where(pos >= DIL * w, l, -1e9 * LOG2E) for w, l in enumerate(lg)]
                top = functools.reduce(jnp.maximum, lg)
                p = [jnp.exp2(l - top) for l in lg]
                g = 1.0 / (1.0 + jnp.exp(-buf[_GATE, rows_at(r0 + h * 8, 8), :]))
                g_v[pl.ds(pl.multiple_of(r0 + h * 8, 8), 8), :] = g
                norm = (1.0 - g) / functools.reduce(jnp.add, p)
                outs = []
                for c in range(NT):
                    pacer.tick(17)
                    acc = None
                    for w in range(WIN):
                        term = p[w] * buf[_V + c, pl.ds(HALO + r0 + h * 8 - DIL * w, 8), :]
                        acc = term if acc is None else acc + term
                    outs.append(acc * norm)
                halves.append(outs)
            for c in range(NT):
                o_v[v, pl.ds(pl.multiple_of((i * steps + n) * 16, 16), 16), _tile(c)] = (
                    jnp.concatenate([halves[0][c], halves[1][c]], axis=0).astype(bf16))

        units, lag = steps * NT, 4
        jobs, ready, prods = sum((gate_sums(n) for n in range(4)), []), [], []
        for u in range(units + lag):
            while len(ready) < min(4 * steps, 4 + 2 * u, 12 + u * 4 // NT):
                jobs += head_sums((len(ready) // 4 + early) % steps, len(ready) % 4)
                ready.append(len(jobs))
            if u < units:
                prod, more = forward(*divmod(u, NT))
                prods.append(prod)
                jobs += more
            if u >= lag:
                jobs += inverse(*divmod(u - lag, NT), prods[u - lag])

        def store_round(group, s):
            for fn in [fn for keep, fn in group if keep] or [group[0][1]]:
                fn(s)

        stores = [functools.partial(store_round, jobs[r:r + 4], s)
                  for r in range(0, len(jobs), 4) for s in range(4)]
        pacer.start(stores, ((steps - early) * score_ops + steps * 8 * (36 + NT * 17)) * 1.04)
        later = [2, 3, 5, 7]
        for m in range(steps):
            for v in range(4):
                pacer.emit(-(-ready[4 * m + v] // 4) * 4)
                attend((m + early) % steps, v)
            if m in later:
                scores(jnp.minimum(i + 1, NI - 1), early + later.index(m))
        pacer.flush()
        return carry

    for n in range(early, steps):
        scores(0, n)
    jax.lax.fori_loop(0, NI, m_step, 0)

    def w_step(i, carry):
        zero = (i // NI) * 8
        fft = _Fft(pacer, lambda k: misc(_COS + k, zero))
        mm = lambda rows, k, n: jnp.dot(o_v[i, rows, k], wop_v[k, n], preferred_element_type=f32)
        stores = matmul_stores(mm, _PROJ, zero)
        pacer.start(stores, NT * (2 * 452 + NA * 15) * 1.15)

        signs = [None, None]

        def mix(c):
            skip_c = misc(_SKIP + c, zero)
            skip_c = jnp.concatenate([skip_c, skip_c], axis=0)
            for a in range(NA):
                pacer.tick(13)
                pacer.emit(len(stores) - (NT - c) * TM // 32 + a // 2 + 1)
                row = pl.multiple_of(a * NB + i * 16, 16)
                staged = pl.ds(pl.multiple_of(2 * zero + a * 16, 8), 16)
                y = (buf[_KV + c, rows_at(row, 16), :] * skip_c, 1)
                for half in range(2):
                    y = fft.add(y, (y32[half, c, staged, :], signs[half][a]))
                y = _value(y)
                branch = y * x_v[pl.ds(row, 16), _tile(c)].astype(f32)
                out_v[i, a, :, _tile(c)] = (
                    branch * g_v[pl.ds(row, 16), :]
                    + buf[_PROJ + c, rows_at(zero + a * 16, 16), :]).astype(bf16)

        for c in range(NT):
            for h in range(2):
                def load(j):
                    pacer.tick()
                    plane = _SPEC + NT * (j // (NA // 2)) + c
                    row = (j % (NA // 2)) * 2 * NB + (2 * i + h) * 16
                    return ((buf[plane, rows_at(row, 8), :], 1), (buf[plane, rows_at(row + 8, 8), :], 1))

                blocks = [functools.partial(load, j) for j in range(NA)]
                for half, fn in enumerate((fft.odd_bwd, fft.even_bwd)):
                    outs = fn(blocks[half * NA // 2:(half + 1) * NA // 2])
                    signs[half] = [sign for _, sign in outs]
                    for a, (val, _) in enumerate(outs):
                        y32[half, c, pl.ds(pl.multiple_of(zero + a * 16 + h * 8, 8), 8), :] = val
            if c >= 2:
                mix(c - 2)
        mix(NT - 2)
        mix(NT - 1)
        pacer.flush()
        out_copy(i).start()
        return carry

    jax.lax.fori_loop(0, NI, w_step, 0)
    for i in range(NI):
        out_copy(i).wait()


@jax.jit
def pallas_gated_mix__ssm_conv_h3__sliding_local_dilated__prompt_kernel(
    A_q: jax.Array,
    A_k: jax.Array,
    A_v: jax.Array,
    A_shift_k: jax.Array,
    A_ssm_k: jax.Array,
    A_ssm_D: jax.Array,
    B_x: jax.Array,
    B_wqkv: jax.Array,
    B_wo: jax.Array,
    gate_w: jax.Array,
):
    del B_x
    assert A_q.shape == (1, S, D) and A_shift_k.shape == (D, KS)
    f32, bf16 = jnp.float32, jnp.bfloat16
    gf, gi = _dft_matrices()
    hbm = pl.BlockSpec(memory_space=pl.ANY)
    vmem = pl.BlockSpec(memory_space=pltpu.VMEM)
    out = pl.pallas_call(
        _kernel,
        out_shape=jax.ShapeDtypeStruct((NA, NB, D), bf16),
        in_specs=[hbm, hbm, hbm, vmem, hbm, vmem, hbm, hbm, vmem, hbm, hbm],
        out_specs=hbm,
        scratch_shapes=[
            pltpu.VMEM((S, D), bf16),
            pltpu.VMEM((S, D), bf16),
            pltpu.VMEM((S, D), bf16),
            pltpu.VMEM((D, S), bf16),
            pltpu.VMEM((3, D, D), bf16),
            pltpu.VMEM((3, D, D), bf16),
            pltpu.VMEM((D, D), bf16),
            pltpu.VMEM((D, D), bf16),
            pltpu.VMEM((NT, D // 2, LANES), jnp.uint32),
            pltpu.VMEM((NA, 2 * NB, 2 * NB), bf16),
            pltpu.VMEM((NA, 2 * NB, 2 * NB), bf16),
            pltpu.VMEM((_LOGITS + 2, HALO + S, LANES), f32),
            pltpu.VMEM((S, LANES), bf16),
            pltpu.VMEM((S, LANES), f32),
            pltpu.VMEM((NA, 2 * NB, 2 * D), bf16),
            pltpu.VMEM((NA // 2, WIN * NB, LANES), bf16),
            pltpu.VMEM((NA // 2, WIN * NB, LANES), bf16),
            pltpu.VMEM((2, NT, TM, LANES), f32),
            pltpu.VMEM((NI, TM, D), bf16),
            pltpu.VMEM((NI, NA, 16, D), bf16),
            pltpu.SemaphoreType.DMA((9,)),
            pltpu.SemaphoreType.DMA((NI,)),
            pltpu.SemaphoreType.DMA((NI,)),
        ],
        compiler_params=pltpu.CompilerParams(vmem_limit_bytes=110 * 1024 * 1024),
        name="gated_mix_h3_local_attn",
    )(A_q.reshape(S, D), A_k.reshape(S, D), A_v.reshape(S, D), A_shift_k.T, A_ssm_k,
      A_ssm_D, B_wqkv, B_wo, gate_w, gf, gi)
    return out.reshape(1, S, D)
```

```python
import functools
import math

import jax
import jax.numpy as jnp
import numpy as np
from jax.experimental import pallas as pl
from jax.experimental.pallas import tpu as pltpu

S = 2048
D = 640
H = 32
DH = D // H
WIN = 8
DIL = 2
KS = 4
LANES = 128
NT = D // LANES
NA = 32
NB = 64
HALO = 16
TM = 512
NI = S // TM


class _Pacer:
    def __init__(self):
        self.stores, self.done, self.ops, self.rate = [], 0, 0, 0.0

    def start(self, stores, vector_ops):
        self.flush()
        self.stores, self.done, self.ops = list(stores), 0, 0
        self.rate = len(self.stores) / vector_ops

    def tick(self, ops=0):
        self.emit(min(len(self.stores), int(self.ops * self.rate)))
        self.ops += ops

    def flush(self):
        self.emit(len(self.stores))

    def emit(self, due):
        while self.done < due:
            self.stores[self.done]()
            self.done += 1


def _neg(a):
    return (a[0], -a[1])


def _mul_i(x, s):
    return (_neg(x[1]), x[0]) if s > 0 else (x[1], _neg(x[0]))


class _Fft:
    def __init__(self, pacer, cosine):
        self.pacer = pacer
        self.cosine = cosine

    def add(self, a, b):
        self.pacer.ops += 1
        if a[1] == b[1]:
            return (a[0] + b[0], a[1])
        return (a[0] - b[0], 1) if a[1] > 0 else (b[0] - a[0], 1)

    def sub(self, a, b):
        return self.add(a, _neg(b))

    def mul(self, a, c):
        self.pacer.ops += 1
        return (a[0] * c[0], a[1] * c[1])

    def cadd(self, x, y):
        return (self.add(x[0], y[0]), self.add(x[1], y[1]))

    def csub(self, x, y):
        return (self.sub(x[0], y[0]), self.sub(x[1], y[1]))

    def cos(self, k):
        k = min(k % 64, -k % 64)
        return (self.cosine(k), 1) if k < 16 else (self.cosine(32 - k), -1)

    def twiddle(self, x, num, den):
        k = (num * (64 // den)) % 64
        if k % 16 == 0:
            for _ in range(k // 16):
                x = _mul_i(x, 1)
            return x
        self.pacer.tick()
        re, im = x
        c = self.cos(k)
        if k % 8 == 0:
            sc, ss = c[1], (1 if k < 32 else -1)
            pick = lambda v, sign: v if sign > 0 else _neg(v)
            return (self.mul(self.sub(pick(re, sc), pick(im, ss)), (c[0], 1)),
                    self.mul(self.add(pick(re, ss), pick(im, sc)), (c[0], 1)))
        s = self.cos(k - 16)
        return (self.sub(self.mul(re, c), self.mul(im, s)),
                self.add(self.mul(re, s), self.mul(im, c)))

    def cfft(self, z, sgn):
        n = len(z)
        if n == 1:
            return [z[0]()]
        if n == 2:
            a, b = z[0](), z[1]()
            return [self.cadd(a, b), self.csub(a, b)]
        ev, o1, o3 = self.cfft(z[0::2], sgn), self.cfft(z[1::4], sgn), self.cfft(z[3::4], sgn)
        out = [None] * n
        for r in range(n // 4):
            t1 = self.twiddle(o1[r], sgn * r, n)
            t3 = self.twiddle(o3[r], sgn * 3 * r, n)
            p, m = self.cadd(t1, t3), _mul_i(self.csub(t1, t3), sgn)
            lo, hi = ev[r], ev[r + n // 4]
            out[r], out[r + n // 2] = self.cadd(lo, p), self.csub(lo, p)
            out[r + n // 4], out[r + 3 * n // 4] = self.cadd(hi, m), self.csub(hi, m)
        return out

    def odd_fwd(self, d):
        m = len(d)
        return self.cfft([lambda a=a: self.twiddle((d[a](), _neg(d[a + m // 2]())), -a, 2 * m)
                          for a in range(m // 2)], -1)

    def odd_bwd(self, y):
        m = 2 * len(y)
        z = [self.twiddle(v, a, 2 * m) for a, v in enumerate(self.cfft(y, 1))]
        return [v[0] for v in z] + [_neg(v[1]) for v in z]

    def even_fwd(self, u):
        n = len(u)
        if n == 2:
            return [(u[0](), u[1]())]
        sums = [None] * (n // 2)

        def diff(a):
            lo, hi = u[a](), u[a + n // 2]()
            sums[a] = self.add(lo, hi)
            return self.sub(lo, hi)

        odd = self.odd_fwd([lambda a=a: diff(a) for a in range(n // 2)])
        return odd + self.even_fwd([lambda v=v: v for v in sums])

    def even_bwd(self, y):
        n = 2 * len(y)
        if n == 2:
            return list(y[0]())
        s, d = self.even_bwd(y[n // 4:]), self.odd_bwd(y[:n // 4])
        return [self.add(a, b) for a, b in zip(s, d)] + [self.sub(a, b) for a, b in zip(s, d)]


def _block_freqs():
    freqs = [4 * r + 1 for r in range(NA // 2)]
    n = NA
    while n > 2:
        freqs += [(4 * r + 1) * (2 * NA // n) for r in range(n // 4)]
        n //= 2
    return freqs + [None]


def _dft_matrices():
    fft = _Fft(_Pacer(), lambda k: 1.0)
    probe = [lambda: (1.0, 1)] * NA
    signs = [(re[1], im[1]) for re, im in fft.odd_fwd(probe) + fft.even_fwd(probe)]
    n = 2 * S
    b = np.arange(NB)
    k2 = np.arange(NB)[:, None]
    fwd = np.zeros((NA, 2 * NB, 2, NB))
    inv = np.zeros((NA, 2 * NB, 2, NB))
    for j, f in enumerate(_block_freqs()):
        weight = np.full((2 * NB, 1), 2.0 / n)
        if f is None:
            for part in range(2):
                ang = -2 * np.pi * ((k2 * (b + NB * part)) % (2 * NB)) / (2 * NB)
                fwd[j, :NB, part], fwd[j, NB:, part] = np.cos(ang), np.sin(ang)
                fwd[j, NB, part] = 1.0 - 2.0 * (b % 2)
            weight[0] = weight[NB] = 1.0 / n
        else:
            ang = -2 * np.pi * ((b * (f + 2 * NA * k2)) % n) / n
            fwd[j, :NB, 0], fwd[j, :NB, 1] = np.cos(ang), -np.sin(ang)
            fwd[j, NB:, 0], fwd[j, NB:, 1] = np.sin(ang), np.cos(ang)
        inv[j] = fwd[j] * weight[:, :, None]
        fwd[j] *= np.asarray(signs[j], np.float64)[None, :, None]
    order = lambda g: g.reshape(NA, 2, NB // 8, 8, 2, NB // 8, 8).transpose(
        0, 2, 1, 3, 5, 4, 6).reshape(NA, 2 * NB, 2 * NB)
    return (order(fwd).astype(jnp.bfloat16),
            order(inv).transpose(0, 2, 1).astype(jnp.bfloat16))


def _value(a):
    return a[0] if a[1] > 0 else -a[0]


_Q, _K, _V, _FILT, _AK, _KV, _MISC = (n * NT for n in range(7))
_GATE = _MISC + 1
_LOGITS = _MISC + 2
_SPEC = _FILT
_PROJ = _Q
_COS, _TAP, _SKIP, _GW, _DUMMY = 0, 16, 16 + KS * NT, 16 + (KS + 1) * NT, 16 + (KS + 2) * NT
LOG2E = math.log2(math.e)


def _tile(c):
    return slice(c * LANES, (c + 1) * LANES)


def _kernel(x_hbm, ak_hbm, av_hbm, shift_ref, ssmk_hbm, d_ref, wqkv_hbm, wo_hbm, gw_ref,
            gf_hbm, gi_hbm, out_hbm,
            x_v, ak_v, av_v, ssmk_v, w_v, wt_v, wo_v, wop_v, words, gf_v, gi_v,
            buf, gate_v, g_v, res, part_a, part_b, y32, o_v, out_v, sem_in, sem_x, sem_out):
    f32, bf16 = jnp.float32, jnp.bfloat16
    pacer = _Pacer()

    def w_copy(p):
        return pltpu.make_async_copy(wqkv_hbm.at[:, pl.ds(p * D, D)], w_v.at[p], sem_in.at[p])

    def x_copy(i):
        rows = pl.ds(pl.multiple_of(i * TM, TM), TM)
        return pltpu.make_async_copy(x_hbm.at[rows], x_v.at[rows], sem_x.at[i])

    ssmk_copy = pltpu.make_async_copy(ssmk_hbm, ssmk_v, sem_in.at[3])
    ak_copy = pltpu.make_async_copy(ak_hbm, ak_v, sem_in.at[4])
    av_copy = pltpu.make_async_copy(av_hbm, av_v, sem_in.at[5])
    gf_copy = pltpu.make_async_copy(gf_hbm, gf_v, sem_in.at[6])
    gi_copy = pltpu.make_async_copy(gi_hbm, gi_v, sem_in.at[7])
    wo_copy = pltpu.make_async_copy(wo_hbm, wo_v, sem_in.at[8])

    def out_copy(i):
        rows = pl.ds(pl.multiple_of(i * 16, 16), 16)
        return pltpu.make_async_copy(out_v.at[i], out_hbm.at[:, rows, :], sem_out.at[i])

    def rows_at(start, size):
        return pl.ds(pl.multiple_of(HALO + start, 8), size)

    def misc(reg, zero):
        return buf[_MISC, pl.ds(pl.multiple_of(zero + reg * 8, 8), 8), :]

    def reorder_rows(tile, dst, u):
        words[u] = pltpu.bitcast(tile, jnp.uint32)
        for pair in range(DH // 2):
            dst[pair * 2 * H:(pair + 1) * 2 * H, _tile(u)] = pltpu.bitcast(
                words[u, pl.ds(pair, H, stride=DH // 2), :], bf16)

    def prepare_weight(p):
        for u in range(NT):
            reorder_rows(w_v[p, _tile(u), :].T, wt_v.at[p], u)

    def matmul_stores(mm, plane, r0, scale=None, group=32):
        k_head, k_tail, quarter = slice(0, D - LANES), slice(D - LANES, D), TM // 4
        staged = mm(slice(0, TM), k_tail, k_head)
        last = [mm(slice(n * quarter, (n + 1) * quarter), k_tail, k_tail) for n in range(4)]
        full = [mm(slice(0, TM), k_head, _tile(c)) for c in range(NT)]

        def stage(v):
            for c in range(NT - 1):
                buf[plane + c, rows_at(r0 + v * group, group), :] = staged[v * group:(v + 1) * group, _tile(c)]

        def stage_last(v):
            for n in range(4):
                buf[plane + NT - 1, rows_at(r0 + n * quarter + v * group, group), :] = (
                    last[n][v * group:(v + 1) * group])

        def finish(c, v):
            rows = rows_at(r0 + v * group, group)
            val = full[c][v * group:(v + 1) * group] + buf[plane + c, rows, :]
            buf[plane + c, rows, :] = val if scale is None else val * scale

        return ([functools.partial(stage, v) for v in range(TM // group)]
                + [functools.partial(stage_last, v) for v in range(quarter // group)]
                + [functools.partial(finish, c, v) for c in range(NT) for v in range(TM // group)])

    lane_head = lambda axis: (jax.lax.broadcasted_iota(jnp.int32, (LANES, LANES), axis) % (2 * H)) // 2

    def gate(i, zero, v):
        pacer.tick(30)
        rows = pl.ds(pl.multiple_of(i * TM + v * 16, 16), 16)
        xs = x_v[rows, :].astype(f32)
        acc = None
        for c in range(NT):
            gw = misc(_GW + c, zero)
            term = xs[:, _tile(c)] * jnp.concatenate([gw, gw], axis=0)
            acc = term if acc is None else acc + term
        gate_v[rows, :] = acc.astype(bf16)

    def first_stage(plane, col, pair, zero, side, chunks=1):
        fft = _Fft(pacer, lambda k: misc(_COS + k, zero))
        for slot in range(2 * NT):
            if slot % (2 * NT // chunks) == 0:
                n = slot // (2 * NT // chunks)
                for job in side[n * len(side) // chunks:(n + 1) * len(side) // chunks]:
                    job()
            beta, c = 2 * pair + slot // NT, slot % NT
            r0 = pl.multiple_of(beta * 16, 16)

            def load(a):
                pacer.tick()
                return (buf[plane + c, rows_at(a * NB + beta * 8, 8), :], 1)

            for half, fn in enumerate((fft.odd_fwd, fft.even_fwd)):
                outs = fn([functools.partial(load, a) for a in range(NA)])
                for j, (re, im) in enumerate(outs):
                    res[half * (NA // 2) + j, pl.ds(r0, 16), _tile(2 * c + col)] = (
                        jnp.concatenate([re[0], im[0]], axis=0).astype(bf16))

    def widen_k(r0):
        pacer.tick(30)
        wide = ak_v[pl.ds(pl.multiple_of(r0, 32), 32), :].astype(f32)
        for c in range(NT):
            buf[_AK + c, rows_at(r0, 32), :] = wide[:, _tile(c)]

    def shift_conv(r0, zero):
        for v in range(2 * TM // 16):
            row = pl.multiple_of(r0 + v * 16, 16)
            vals = av_v[pl.ds(row, 16), :].astype(f32)
            kv = []
            for c in range(NT):
                pacer.tick(19)
                acc = None
                for t in range(KS):
                    tap = misc(_TAP + t * NT + c, zero)
                    term = (buf[_AK + c, pl.ds(HALO + row - t, 16), :]
                            * jnp.concatenate([tap, tap], axis=0))
                    acc = term if acc is None else acc + term
                kv.append(acc * vals[:, _tile(c)])
            for c in range(NT):
                buf[_KV + c, rows_at(row, 16), :] = kv[c]

    def part(i, n):
        return (part_a if n < early else part_b).at[i * early + n % early]

    def scores(i, n, groups=range(4)):
        for v in groups:
            r0 = i * TM + n * NB + v * 16
            q = [buf[_Q + c, rows_at(r0, 16), :] for c in range(NT)]
            for w in range(WIN):
                pacer.tick(19)
                acc = None
                for c in range(NT):
                    term = q[c] * buf[_K + c, pl.ds(HALO + r0 - DIL * w, 16), :]
                    acc = term if acc is None else acc + term
                part(i, n)[(v * WIN + w) * 16:(v * WIN + w + 1) * 16, :] = acc.astype(bf16)

    gate_ops, stage_ops, score_ops = TM // 16 * 30, NT * 452, 4 * WIN * 19
    steps = NA // NI
    early = steps // 2

    def projection(p, plane, lo, hi, vector_ops, work, scale=None, group=32):
        def step(i, carry):
            if p == 0:
                x_copy(i).wait()
            r0 = pl.multiple_of(i * TM, TM)

            def mm(rows, k, n):
                lhs = x_v[pl.ds(r0 + rows.start, rows.stop - rows.start), k]
                return jax.lax.dot_general(lhs, wt_v[p, n, k], (((1,), (1,)), ((), ())),
                                           preferred_element_type=f32)

            pacer.start(matmul_stores(mm, plane, r0, scale, group), vector_ops * 1.02)
            work(i, (i // NI) * 8)
            pacer.flush()
            return carry

        jax.lax.fori_loop(lo, hi, step, 0)

    def fill_halo(plane):
        for c in range(NT):
            buf[plane + c, 0:HALO, :] = jnp.broadcast_to(buf[plane + c, HALO:HALO + 1, :], (HALO, LANES))

    for cp in (w_copy(0), x_copy(0)):
        cp.start()
    for k in range(1, 16):
        buf[_MISC, (_COS + k) * 8:(_COS + k + 1) * 8, :] = jnp.full(
            (8, LANES), math.cos(2 * math.pi * k / 64), f32)
    rows = [shift_ref[...].astype(f32)[t:t + 1] for t in range(KS)]
    rows += [d_ref[...].astype(f32).reshape(1, D), gw_ref[...].astype(f32).reshape(1, D)]
    for c in range(NT):
        for n, row in enumerate(rows):
            reg = _TAP + n * NT + c
            buf[_MISC, reg * 8:(reg + 1) * 8, :] = jnp.broadcast_to(row[:, _tile(c)], (8, LANES))
        buf[_AK + c, 0:HALO, :] = jnp.zeros((HALO, LANES), f32)
    w_copy(0).wait()
    x_copy(1).start()
    prepare_weight(0)

    q_scale = DH ** -0.5 * LOG2E
    ssmk_copy.start()
    gates = lambda i, zero: [functools.partial(gate, i, zero, v) for v in range(TM // 16)]
    projection(0, _Q, 0, NI // 2, gate_ops, lambda i, zero: [job() for job in gates(i, zero)], q_scale)
    ssmk_copy.wait()
    for cp in (x_copy(2), x_copy(3), w_copy(1)):
        cp.start()
    for c in range(NT):
        for t in range(S // 256):
            buf[_FILT + c, HALO + t * 256:HALO + (t + 1) * 256, :] = (
                ssmk_v[_tile(c), t * 256:(t + 1) * 256].T.astype(f32))
    ak_copy.start()

    def q_work(i, zero):
        first_stage(_FILT, 1, i - NI // 2, zero, gates(i, zero))

    projection(0, _Q, NI // 2, NI, gate_ops + 2 * stage_ops, q_work, q_scale)

    for cp in (av_copy, w_copy(2)):
        cp.start()
    w_copy(1).wait()
    prepare_weight(1)
    ak_copy.wait()

    def k_work(i, zero):
        first_stage(_FILT, 1, NI // 2 + i, zero,
                    [functools.partial(widen_k, i * 2 * TM + v * 32) for v in range(2 * TM // 32)])

    projection(1, _K, 0, NI // 2, 2 * TM // 32 * 30 + 2 * stage_ops, k_work)
    for cp in (gf_copy, gi_copy, wo_copy):
        cp.start()
    av_copy.wait()
    projection(1, _K, NI // 2, NI, 2 * TM // 16 * NT * 19,
               lambda i, zero: shift_conv((i - NI // 2) * 2 * TM, zero), group=64)
    fill_halo(_K)

    w_copy(2).wait()
    prepare_weight(2)

    def v_work(i, zero):
        first_stage(_KV, 0, i, zero,
                    [functools.partial(scores, i, n, [v]) for n in range(early) for v in range(4)], 2)

    projection(2, _V, 0, NI, 2 * stage_ops + early * score_ops, v_work)
    fill_halo(_V)

    gf_copy.wait()
    gi_copy.wait()
    wo_copy.wait()
    for u in range(NT):
        reorder_rows(wo_v[:, _tile(u)], wop_v, u)

    def m_step(i, carry):
        zero = (i // NI) * 8
        same_head = (lane_head(0) == lane_head(1)).astype(bf16)

        def logit_rows(n, start, size):
            return _LOGITS + n // 4, rows_at(zero + (n % 4) * WIN * NB + start, size)

        def head_sums(n, v):
            logits = jnp.dot(part(i, n)[v * 2 * NB:(v + 1) * 2 * NB, :], same_head,
                             preferred_element_type=f32)

            def put(s):
                plane, rows = logit_rows(n, v * 2 * NB + s * 32, 32)
                buf[plane, rows, :] = logits[s * 32:(s + 1) * 32]
            return [(True, put)]

        def gate_sums(n):
            r0 = i * TM + n * 2 * NB
            z = jnp.dot(gate_v[pl.ds(pl.multiple_of(r0, 2 * NB), 2 * NB), :],
                        jnp.ones((LANES, LANES), bf16), preferred_element_type=f32)

            def put(s):
                buf[_GATE, rows_at(r0 + s * 32, 32), :] = z[s * 32:(s + 1) * 32]
            return [(True, put)]

        def forward(n, c):
            j = i * steps + n
            f = jnp.dot(gf_v[j], res[j, :, 2 * c * LANES:2 * (c + 1) * LANES],
                        preferred_element_type=f32)
            groups = []
            for v in range(NB // 8):
                re, im = slice(v * 16, v * 16 + 8), slice(v * 16 + 8, v * 16 + 16)
                ur, ui, kr, ki = f[re, :LANES], f[im, :LANES], f[re, LANES:], f[im, LANES:]
                rr, ii = ur * kr, ui * ki
                pr, pi = rr - ii, ur * ki + ui * kr
                if n == steps - 1 and v == 0:
                    real = ((jax.lax.broadcasted_iota(jnp.int32, (8, LANES), 0) == 0)
                            & (i == NI - 1))
                    pr, pi = jnp.where(real, rr, pr), jnp.where(real, ii, pi)
                groups += [pr, pi]

            def mark(t, s):
                buf[_MISC, pl.ds(pl.multiple_of(zero + _DUMMY * 8, 8), 8), :] = (
                    f[s * 32 + 24:(s + 1) * 32, _tile(t)])
            return (jnp.concatenate(groups, axis=0).astype(bf16),
                    [(False, functools.partial(mark, t)) for t in range(2)])

        def inverse(n, c, prod):
            j = i * steps + n
            back = jnp.dot(gi_v[j], prod, preferred_element_type=f32)

            def put(s):
                buf[_SPEC + NT * (j // (NA // 2)) + c,
                    rows_at((j % (NA // 2)) * 2 * NB + s * 32, 32), :] = back[s * 32:(s + 1) * 32]
            return [(True, put)]

        def attend(n, v):
            r0 = i * TM + n * NB + v * 16
            halves = []
            for h in range(2):
                pacer.tick(36)
                lg = []
                for w in range(WIN):
                    plane, rows = logit_rows(n, (v * WIN + w) * 16 + h * 8, 8)
                    lg.append(buf[plane, rows, :])
                if n == 0 and v == 0:
                    pos = r0 + h * 8 + jax.lax.broadcasted_iota(jnp.int32, (8, LANES), 0)
                    lg = [jnp.where(pos >= DIL * w, l, -1e9 * LOG2E) for w, l in enumerate(lg)]
                top = functools.reduce(jnp.maximum, lg)
                p = [jnp.exp2(l - top) for l in lg]
                g = 1.0 / (1.0 + jnp.exp(-buf[_GATE, rows_at(r0 + h * 8, 8), :]))
                g_v[pl.ds(pl.multiple_of(r0 + h * 8, 8), 8), :] = g
                norm = (1.0 - g) / functools.reduce(jnp.add, p)
                outs = []
                for c in range(NT):
                    pacer.tick(17)
                    acc = None
                    for w in range(WIN):
                        term = p[w] * buf[_V + c, pl.ds(HALO + r0 + h * 8 - DIL * w, 8), :]
                        acc = term if acc is None else acc + term
                    outs.append(acc * norm)
                halves.append(outs)
            for c in range(NT):
                o_v[v, pl.ds(pl.multiple_of((i * steps + n) * 16, 16), 16), _tile(c)] = (
                    jnp.concatenate([halves[0][c], halves[1][c]], axis=0).astype(bf16))

        units, lag = steps * NT, 4
        jobs, ready, prods = sum((gate_sums(n) for n in range(4)), []), [], []
        for u in range(units + lag):
            while len(ready) < min(4 * steps, 4 + 2 * u, 12 + u * 4 // NT):
                jobs += head_sums((len(ready) // 4 + early) % steps, len(ready) % 4)
                ready.append(len(jobs))
            if u < units:
                prod, more = forward(*divmod(u, NT))
                prods.append(prod)
                jobs += more
            if u >= lag:
                jobs += inverse(*divmod(u - lag, NT), prods[u - lag])

        def store_round(group, s):
            for fn in [fn for keep, fn in group if keep] or [group[0][1]]:
                fn(s)

        stores = [functools.partial(store_round, jobs[r:r + 4], s)
                  for r in range(0, len(jobs), 4) for s in range(4)]
        pacer.start(stores, ((steps - early) * score_ops + steps * 8 * (36 + NT * 17)) * 1.04)
        later = [2, 3, 5, 7]
        for m in range(steps):
            for v in range(4):
                pacer.emit(-(-ready[4 * m + v] // 4) * 4)
                attend((m + early) % steps, v)
            if m in later:
                scores(jnp.minimum(i + 1, NI - 1), early + later.index(m))
        pacer.flush()
        return carry

    for n in range(early, steps):
        scores(0, n)
    jax.lax.fori_loop(0, NI, m_step, 0)

    def w_step(i, carry):
        zero = (i // NI) * 8
        fft = _Fft(pacer, lambda k: misc(_COS + k, zero))
        mm = lambda rows, k, n: jnp.dot(o_v[i, rows, k], wop_v[k, n], preferred_element_type=f32)
        stores = matmul_stores(mm, _PROJ, zero)
        pacer.start(stores, NT * (2 * 452 + NA * 15) * 1.15)

        signs = [None, None]

        def mix(c):
            skip_c = misc(_SKIP + c, zero)
            skip_c = jnp.concatenate([skip_c, skip_c], axis=0)
            for a in range(NA):
                pacer.tick(13)
                pacer.emit(len(stores) - (NT - c) * TM // 32 + a // 2 + 1)
                row = pl.multiple_of(a * NB + i * 16, 16)
                staged = pl.ds(pl.multiple_of(2 * zero + a * 16, 8), 16)
                y = (buf[_KV + c, rows_at(row, 16), :] * skip_c, 1)
                for half in range(2):
                    y = fft.add(y, (y32[half, c, staged, :], signs[half][a]))
                y = _value(y)
                branch = y * x_v[pl.ds(row, 16), _tile(c)].astype(f32)
                out_v[i, a, :, _tile(c)] = (
                    branch * g_v[pl.ds(row, 16), :]
                    + buf[_PROJ + c, rows_at(zero + a * 16, 16), :]).astype(bf16)

        for c in range(NT):
            for h in range(2):
                def load(j):
                    pacer.tick()
                    plane = _SPEC + NT * (j // (NA // 2)) + c
                    row = (j % (NA // 2)) * 2 * NB + (2 * i + h) * 16
                    return ((buf[plane, rows_at(row, 8), :], 1), (buf[plane, rows_at(row + 8, 8), :], 1))

                blocks = [functools.partial(load, j) for j in range(NA)]
                for half, fn in enumerate((fft.odd_bwd, fft.even_bwd)):
                    outs = fn(blocks[half * NA // 2:(half + 1) * NA // 2])
                    signs[half] = [sign for _, sign in outs]
                    for a, (val, _) in enumerate(outs):
                        y32[half, c, pl.ds(pl.multiple_of(zero + a * 16 + h * 8, 8), 8), :] = val
            if c >= 2:
                mix(c - 2)
        mix(NT - 2)
        mix(NT - 1)
        pacer.flush()
        out_copy(i).start()
        return carry

    jax.lax.fori_loop(0, NI, w_step, 0)
    for i in range(NI):
        out_copy(i).wait()


@jax.jit
def pallas_gated_mix__ssm_conv_h3__sliding_local_dilated__prompt_kernel(
    A_q: jax.Array,
    A_k: jax.Array,
    A_v: jax.Array,
    A_shift_k: jax.Array,
    A_ssm_k: jax.Array,
    A_ssm_D: jax.Array,
    B_x: jax.Array,
    B_wqkv: jax.Array,
    B_wo: jax.Array,
    gate_w: jax.Array,
):
    del B_x
    assert A_q.shape == (1, S, D) and A_shift_k.shape == (D, KS)
    f32, bf16 = jnp.float32, jnp.bfloat16
    gf, gi = _dft_matrices()
    hbm = pl.BlockSpec(memory_space=pl.ANY)
    vmem = pl.BlockSpec(memory_space=pltpu.VMEM)
    out = pl.pallas_call(
        _kernel,
        out_shape=jax.ShapeDtypeStruct((NA, NB, D), bf16),
        in_specs=[hbm, hbm, hbm, vmem, hbm, vmem, hbm, hbm, vmem, hbm, hbm],
        out_specs=hbm,
        scratch_shapes=[
            pltpu.VMEM((S, D), bf16),
            pltpu.VMEM((S, D), bf16),
            pltpu.VMEM((S, D), bf16),
            pltpu.VMEM((D, S), bf16),
            pltpu.VMEM((3, D, D), bf16),
            pltpu.VMEM((3, D, D), bf16),
            pltpu.VMEM((D, D), bf16),
            pltpu.VMEM((D, D), bf16),
            pltpu.VMEM((NT, D // 2, LANES), jnp.uint32),
            pltpu.VMEM((NA, 2 * NB, 2 * NB), bf16),
            pltpu.VMEM((NA, 2 * NB, 2 * NB), bf16),
            pltpu.VMEM((_LOGITS + 2, HALO + S, LANES), f32),
            pltpu.VMEM((S, LANES), bf16),
            pltpu.VMEM((S, LANES), f32),
            pltpu.VMEM((NA, 2 * NB, 2 * D), bf16),
            pltpu.VMEM((NA // 2, WIN * NB, LANES), bf16),
            pltpu.VMEM((NA // 2, WIN * NB, LANES), bf16),
            pltpu.VMEM((2, NT, TM, LANES), f32),
            pltpu.VMEM((NI, TM, D), bf16),
            pltpu.VMEM((NI, NA, 16, D), bf16),
            pltpu.SemaphoreType.DMA((9,)),
            pltpu.SemaphoreType.DMA((NI,)),
            pltpu.SemaphoreType.DMA((NI,)),
        ],
        compiler_params=pltpu.CompilerParams(vmem_limit_bytes=110 * 1024 * 1024),
        name="gated_mix_h3_local_attn",
    )(A_q.reshape(S, D), A_k.reshape(S, D), A_v.reshape(S, D), A_shift_k.T, A_ssm_k,
      A_ssm_D, B_wqkv, B_wo, gate_w, gf, gi)
    return out.reshape(1, S, D)
```
